```python
import jax
import jax.numpy as jnp

def _softmax(x, axis=-1):
    return jax.nn.softmax(x, axis=axis)

def _gelu(x):
    return jax.nn.gelu(x, approximate=True)

def _silu(x):
    return jax.nn.silu(x)

def _sigmoid(x):
    return jax.nn.sigmoid(x)

def _layernorm(x, axis=-1, eps=1e-05):
    m = jnp.mean(x, axis=axis, keepdims=True)
    v = jnp.var(x, axis=axis, keepdims=True)
    return (x - m) / jnp.sqrt(v + eps)

def _scatter_add(tgt, idx, src, axis=0):
    return tgt.at[idx].add(src)

def _segment_sum(src, seg, n):
    return jax.ops.segment_sum(src, seg, n)

class _Rng:

    def __init__(self, key):
        self._k = key

    def _next(self):
        self._k, sub = jax.random.split(self._k)
        return sub

    def normal(self, shape):
        return jax.random.normal(self._next(), shape, dtype=jnp.bfloat16)

    def randint(self, lo, hi, shape):
        return jax.random.randint(self._next(), shape, lo, hi, dtype=jnp.int32)

    def uniform(self, shape, lo=0.0, hi=1.0):
        return jax.random.uniform(self._next(), shape, jnp.bfloat16, lo, hi)

    def permutation(self, n):
        return jax.random.permutation(self._next(), n)
kernel_name = 'gated_mix__memory_aug_recurrent_mem_tr__mixer_s_mlp__prompt'

def setup_inputs():
    _rng = _Rng(jax.random.key(int.from_bytes(__import__("os").urandom(4), "little")))
    _w = lambda a: (lambda t: t.astype(jnp.bfloat16) if jnp.issubdtype(t.dtype, jnp.floating) else t)(jnp.asarray(a))

    def _A_setup():
        B, S, Dm = (1, 2048, 1024)
        H, Dh = (32, 128)
        M, seg = (8, 32)
        seg = min(seg, S)
        S = S // seg * seg
        return {'x': _w((lambda *s: _rng.normal(s) * 0.05)(B, S, Dm)), 'mem0': _w((lambda *s: _rng.normal(s) * 0.05)(B, M, Dm)), 'Wq': _w((lambda *s: _rng.normal(s) * 0.05)(Dm, H, Dh) * Dm ** (-0.5)), 'Wk': _w((lambda *s: _rng.normal(s) * 0.05)(Dm, H, Dh) * Dm ** (-0.5)), 'Wv': _w((lambda *s: _rng.normal(s) * 0.05)(Dm, H, Dh) * Dm ** (-0.5)), 'Wo': _w((lambda *s: _rng.normal(s) * 0.05)(H, Dh, Dm) * (H * Dh) ** (-0.5)), 'seg_len': seg}
    _A_in = _A_setup()

    def _B_setup():
        B, S, D, F = (1, 2048, 1024, 3584)
        return {'x': _w((lambda *s: _rng.normal(s) * 0.05)(B, S, D)), 'w1': _w((lambda *s: _rng.normal(s) * 0.05)(D, D) * D ** (-0.5)), 'w2': _w((lambda *s: _rng.normal(s) * 0.05)(D, D) * D ** (-0.5)), 'w3': _w((lambda *s: _rng.normal(s) * 0.05)(D, F) * D ** (-0.5)), 'w4': _w((lambda *s: _rng.normal(s) * 0.05)(F, D) * F ** (-0.5))}
    _B_in = _B_setup()
    return {'A_x': _A_in['x'], 'A_mem0': _A_in['mem0'], 'A_Wq': _A_in['Wq'], 'A_Wk': _A_in['Wk'], 'A_Wv': _A_in['Wv'], 'A_Wo': _A_in['Wo'], 'A_seg_len': _A_in['seg_len'], 'B_x': _B_in['x'], 'B_w1': _B_in['w1'], 'B_w2': _B_in['w2'], 'B_w3': _B_in['w3'], 'B_w4': _B_in['w4'], 'gate_w': _w((lambda *s: _rng.normal(s) * 0.05)(1024))}

def reference(A_x, A_mem0, A_Wq, A_Wk, A_Wv, A_Wo, A_seg_len, B_x, B_w1, B_w2, B_w3, B_w4, gate_w):

    def _A_ref(x, mem0, Wq, Wk, Wv, Wo, seg_len):
        B, S, Dm = x.shape
        H, Dh = (Wq.shape[1], Wq.shape[2])
        M = mem0.shape[1]
        scale = Dh ** (-0.5)
        n_seg = S // seg_len
        L = M + seg_len
        idx = jnp.arange(L)
        mask = (idx[:, None] < M) | (idx[:, None] >= idx[None, :])
        mem = mem0
        outs = []
        for s in range(n_seg):
            xs = x[:, s * seg_len:(s + 1) * seg_len, :].copy()
            h = jnp.concatenate([mem, xs], axis=1)
            q = jnp.einsum('btd,dhe->bhte', h, Wq)
            k = jnp.einsum('btd,dhe->bhte', h, Wk)
            v = jnp.einsum('btd,dhe->bhte', h, Wv)
            scores = jnp.einsum('bhqe,bhke->bhqk', q, k) * scale
            scores = jnp.where(mask[None, None], scores, -1000000000.0)
            p = _softmax(scores, axis=-1)
            o = jnp.einsum('bhqk,bhke->bhqe', p, v)
            o = jnp.einsum('bhte,hed->btd', o, Wo)
            mem = o[:, :M, :].copy()
            outs.append(o[:, M:, :])
        return jnp.concatenate(outs, axis=1)

    def _B_ref(x, w1, w2, w3, w4):
        B, S, D = x.shape
        h = _gelu(_layernorm(x, axis=-1) @ w1)
        c = D // 4
        g0 = jnp.pad(h[:, :, 0 * c:1 * c], ((0, 0), (1, 0), (0, 0)))[:, :S, :]
        g1 = jnp.pad(h[:, :, 1 * c:2 * c], ((0, 0), (0, 1), (0, 0)))[:, 1:, :]
        g2 = jnp.pad(h[:, :, 2 * c:3 * c], ((0, 0), (2, 0), (0, 0)))[:, :S, :]
        g3 = jnp.pad(h[:, :, 3 * c:], ((0, 0), (0, 2), (0, 0)))[:, 2:, :]
        hs = jnp.concatenate([g0, g1, g2, g3], axis=-1) @ w2
        x1 = x + hs
        h2 = _gelu(_layernorm(x1, axis=-1) @ w3) @ w4
        return x1 + h2
    x = A_x
    g = _sigmoid((x * gate_w).sum(-1, keepdims=True))
    a = _A_ref(x, A_mem0, A_Wq, A_Wk, A_Wv, A_Wo, A_seg_len)
    b = _B_ref(x, B_w1, B_w2, B_w3, B_w4)
    return g * a + (1 - g) * b
```

```python
import functools

import jax
import jax.numpy as jnp
from jax import lax
import jax.experimental.pallas as pl
import jax.experimental.pallas.tpu as pltpu

F32 = jnp.float32
BF16 = jnp.bfloat16
U32 = jnp.uint32

ROWS_B = 256
F_CHUNK = 512
HALO = 8


def _dot(a, b):
    return lax.dot_general(a, b, (((1,), (0,)), ((), ())), preferred_element_type=F32)


def _dot_nt(a, b):
    return lax.dot_general(a, b, (((1,), (1,)), ((), ())), preferred_element_type=F32)


def _layernorm(x, eps=1e-05):
    m = jnp.mean(x, axis=-1, keepdims=True)
    c = x - m
    v = jnp.mean(c * c, axis=-1, keepdims=True)
    return c * lax.rsqrt(v + eps)


def _gelu(x):
    return jax.nn.gelu(x, approximate=True)


def _kernel(ax_hbm, mem0_ref, wq_hbm, wk_hbm, wv_hbm, wo_hbm, w1_hbm, w2_hbm,
            w3_hbm, w4_hbm, gw_ref, out_hbm,
            wqkv, wo, w1, w2, w3, w4, ax, hbuf, bres, gate, hseg, obuf, outbuf,
            sem_in, sem_qkv, sem_wo, sem_out, *, seg):
    S, D = ax.shape
    H, E = wq_hbm.shape[1], wq_hbm.shape[2]
    HP = H // 2
    M = mem0_ref.shape[1]
    L = M + seg
    F = w3.shape[1]
    n_seg = S // seg
    n_tiles = D // 128
    scale = E ** (-0.5)

    cp_w1 = pltpu.make_async_copy(w1_hbm, w1, sem_in.at[1])
    cp_w2 = pltpu.make_async_copy(w2_hbm, w2, sem_in.at[2])
    cp_ax = pltpu.make_async_copy(ax_hbm.at[0], ax, sem_in.at[0])
    cp_w3 = pltpu.make_async_copy(w3_hbm, w3, sem_in.at[4])
    cp_w4 = pltpu.make_async_copy(w4_hbm, w4, sem_in.at[3])
    cp_qkv = [
        pltpu.make_async_copy(w.bitcast(U32).at[:, hp, :], wqkv.at[i * HP + hp],
                              sem_qkv.at[i * HP + hp])
        for i, w in enumerate((wq_hbm, wk_hbm, wv_hbm)) for hp in range(HP)]
    cp_wo = [
        pltpu.make_async_copy(wo_hbm.at[:, :, pl.ds(n * 128, 128)], wo.at[n], sem_wo.at[n])
        for n in range(n_tiles)]
    for cp in (cp_ax, cp_w1, cp_w2, cp_w3, cp_w4):
        cp.start()

    hbuf[0:HALO, :] = jnp.zeros((HALO, D), F32)
    hbuf[HALO + S:, :] = jnp.zeros((HALO, D), F32)
    cp_ax.wait()
    cp_w1.wait()

    def b1_body(i, carry):
        r = pl.multiple_of(i * ROWS_B, ROWS_B)
        x = ax[pl.ds(r, ROWS_B), :].astype(F32)
        h = _gelu(_dot(_layernorm(x).astype(BF16), w1[...]))
        hbuf[pl.ds(pl.multiple_of(r + HALO, 8), ROWS_B), :] = h
        return carry

    lax.fori_loop(0, S // ROWS_B, b1_body, 0)

    cp_w2.wait()
    cp_w3.wait()
    cp_w4.wait()
    for cp in cp_qkv + cp_wo:
        cp.start()

    gw = gw_ref[...].reshape(1, D).astype(F32)
    c = D // 4

    def b2_body(i, carry):
        r = pl.multiple_of(i * ROWS_B, ROWS_B)
        parts = []
        for j, shift in enumerate((-1, 1, -2, 2)):
            win = hbuf[pl.ds(r, ROWS_B + 2 * HALO), pl.ds(j * c, c)]
            parts.append(win[HALO + shift:HALO + shift + ROWS_B].astype(BF16))
        hs = _dot(jnp.concatenate(parts, axis=1), w2[...])
        xa = ax[pl.ds(r, ROWS_B), :].astype(F32)
        x1 = xa + hs
        ln = _layernorm(x1).astype(BF16)
        acc = x1
        for f in range(0, F, F_CHUNK):
            a = _gelu(_dot(ln, w3[:, f:f + F_CHUNK])).astype(BF16)
            acc = acc + _dot(a, w4[f:f + F_CHUNK, :])
        g = jax.nn.sigmoid(jnp.sum(xa * gw, axis=-1, keepdims=True))
        bres[pl.ds(r, ROWS_B), :] = (1.0 - g) * acc
        gate[pl.ds(r, ROWS_B), :] = jnp.broadcast_to(g, (ROWS_B, 128))
        return carry

    lax.fori_loop(0, S // ROWS_B, b2_body, 0)

    for cp in cp_qkv + cp_wo:
        cp.wait()

    def repack(i, carry):
        j = i // n_tiles
        r = pl.multiple_of((i % n_tiles) * 128, 128)
        w = wqkv[j, pl.ds(r, 128), :]
        even = pltpu.bitcast(w << 16, F32).astype(BF16)
        odd = pltpu.bitcast(w & U32(0xFFFF0000), F32).astype(BF16)
        wqkv[j, pl.ds(r, 64), :] = pltpu.bitcast(even, U32)
        wqkv[j, pl.ds(pl.multiple_of(r + 64, 64), 64), :] = pltpu.bitcast(odd, U32)
        return carry

    lax.fori_loop(0, 3 * HP * n_tiles, repack, 0, unroll=4)

    def head_weight(i, h):
        j = i * HP + h // 2
        off = (h % 2) * 64
        w = jnp.concatenate(
            [wqkv[j, k * 128 + off:k * 128 + off + 64, :] for k in range(n_tiles)], axis=0)
        return pltpu.bitcast(w, BF16)

    row = lax.broadcasted_iota(jnp.int32, (L, L), 0)
    col = lax.broadcasted_iota(jnp.int32, (L, L), 1)
    mask = (row < M) | (row >= col)

    hseg[0:M, :] = mem0_ref[0].astype(F32)

    def out_copy(r):
        return pltpu.make_async_copy(outbuf.at[pl.ds(r, seg)], out_hbm.at[0, pl.ds(r, seg)],
                                     sem_out)

    def seg_body(s, carry):
        r = pl.multiple_of(s * seg, seg)
        hseg[M:L, :] = ax[pl.ds(r, seg), :].astype(F32)
        qkv = {}
        probs = {}

        def project(h):
            hh = hseg[...]
            qkv[h] = [_dot(hh, head_weight(i, h)) for i in range(3)]

        def scores(h):
            q, k, _ = qkv[h]
            sc = jnp.where(mask, _dot_nt(q, k) * scale, -1000000000.0)
            e = jnp.exp(sc - jnp.max(sc, axis=-1, keepdims=True))
            probs[h] = (e, jnp.sum(e, axis=-1, keepdims=True))

        def values(h):
            e, den = probs.pop(h)
            v = qkv.pop(h)[2]
            obuf[:, h * E:(h + 1) * E] = _dot(e, v) / den

        def out_part(h0, h1, n):
            w = wo[n, h0:h1].reshape((h1 - h0) * E, 128)
            return _dot(obuf[:, h0 * E:h1 * E], w)

        for h in range(H):
            project(h)
            if h >= 1:
                scores(h - 1)
            if h >= 2:
                values(h - 2)
        half = H // 2
        acc = []
        for n in range(n_tiles):
            acc.append(out_part(0, half, n))
            if n == 0:
                scores(H - 1)
                values(H - 2)
            if n == 2:
                values(H - 1)
        g = gate[pl.ds(r, seg), :]
        for n in range(n_tiles):
            o = acc[n] + out_part(half, H, n)
            cols = slice(n * 128, (n + 1) * 128)
            hseg[0:M, cols] = o[0:M]
            outbuf[pl.ds(r, seg), cols] = (g * o[M:L] + bres[pl.ds(r, seg), cols]).astype(BF16)
        out_copy(r).start()
        return carry

    lax.fori_loop(0, n_seg, seg_body, 0)
    pltpu.make_async_copy(outbuf, out_hbm.at[0], sem_out).wait()


@functools.partial(jax.jit, static_argnames=("A_seg_len",))
def pallas_gated_mix__memory_aug_recurrent_mem_tr__mixer_s_mlp__prompt_kernel(
    A_x: jax.Array,
    A_mem0: jax.Array,
    A_Wq: jax.Array,
    A_Wk: jax.Array,
    A_Wv: jax.Array,
    A_Wo: jax.Array,
    A_seg_len: int,
    B_x: jax.Array,
    B_w1: jax.Array,
    B_w2: jax.Array,
    B_w3: jax.Array,
    B_w4: jax.Array,
    gate_w: jax.Array,
):
    _, S, D = A_x.shape
    _, H, E = A_Wq.shape
    M = A_mem0.shape[1]
    F = B_w3.shape[1]
    seg = int(A_seg_len)
    hbm = pl.BlockSpec(memory_space=pl.ANY)
    vmem = pl.BlockSpec(memory_space=pltpu.VMEM)
    return pl.pallas_call(
        functools.partial(_kernel, seg=seg),
        out_shape=jax.ShapeDtypeStruct(A_x.shape, A_x.dtype),
        in_specs=[hbm, vmem, hbm, hbm, hbm, hbm, hbm, hbm, hbm, hbm, vmem],
        out_specs=hbm,
        scratch_shapes=[
            pltpu.VMEM((3 * H // 2, D, E), U32),
            pltpu.VMEM((D // 128, H, E, 128), BF16),
            pltpu.VMEM((D, D), BF16),
            pltpu.VMEM((D, D), BF16),
            pltpu.VMEM((D, F), BF16),
            pltpu.VMEM((F, D), BF16),
            pltpu.VMEM((S, D), BF16),
            pltpu.VMEM((S + 2 * HALO, D), F32),
            pltpu.VMEM((S, D), F32),
            pltpu.VMEM((S, 128), F32),
            pltpu.VMEM((M + seg, D), F32),
            pltpu.VMEM((M + seg, H * E), F32),
            pltpu.VMEM((S, D), BF16),
            pltpu.SemaphoreType.DMA((5,)),
            pltpu.SemaphoreType.DMA((3 * H // 2,)),
            pltpu.SemaphoreType.DMA((D // 128,)),
            pltpu.SemaphoreType.DMA(()),
        ],
        compiler_params=pltpu.CompilerParams(vmem_limit_bytes=120 * 1024 * 1024),
    )(A_x, A_mem0, A_Wq, A_Wk, A_Wv, A_Wo, B_w1, B_w2, B_w3, B_w4, gate_w)
```

```python
import functools

import jax
import jax.numpy as jnp
from jax import lax
import jax.experimental.pallas as pl
import jax.experimental.pallas.tpu as pltpu

F32 = jnp.float32
BF16 = jnp.bfloat16
U32 = jnp.uint32

ROWS_B = 256
F_CHUNK = 512
HALO = 8


def _dot(a, b):
    return lax.dot_general(a, b, (((1,), (0,)), ((), ())), preferred_element_type=F32)


def _dot_nt(a, b):
    return lax.dot_general(a, b, (((1,), (1,)), ((), ())), preferred_element_type=F32)


def _layernorm(x, eps=1e-05):
    m = jnp.mean(x, axis=-1, keepdims=True)
    c = x - m
    v = jnp.mean(c * c, axis=-1, keepdims=True)
    return c * lax.rsqrt(v + eps)


def _gelu(x):
    return jax.nn.gelu(x, approximate=True)


def _kernel(ax_hbm, mem0_ref, wq_hbm, wk_hbm, wv_hbm, wo_hbm, w1_hbm, w2_hbm,
            w3_hbm, w4_hbm, gw_ref, out_hbm,
            wqkv, wo, w1, w2, w3, w4, ax, hbuf, bres, gate, hseg, obuf, oacc, outbuf,
            sem_in, sem_qkv, sem_out, *, seg):
    S, D = ax.shape
    H, E = wq_hbm.shape[1], wq_hbm.shape[2]
    HP = H // 2
    M = mem0_ref.shape[1]
    L = M + seg
    F = w3.shape[1]
    n_seg = S // seg
    n_tiles = D // 128
    scale = E ** (-0.5)

    n_blk = S // ROWS_B
    cp_x0 = pltpu.make_async_copy(ax_hbm.at[0, 0:ROWS_B], ax.at[0:ROWS_B], sem_in.at[0])
    cp_w1 = pltpu.make_async_copy(w1_hbm, w1, sem_in.at[1])
    cp_x1 = pltpu.make_async_copy(ax_hbm.at[0, ROWS_B:S], ax.at[ROWS_B:S], sem_in.at[2])
    cp_w2 = pltpu.make_async_copy(w2_hbm, w2, sem_in.at[3])
    cp_w3 = pltpu.make_async_copy(w3_hbm, w3, sem_in.at[4])
    cp_w4 = pltpu.make_async_copy(w4_hbm, w4, sem_in.at[5])

    per_blk = HP // n_blk

    def a_copies(i):
        cps = [pltpu.make_async_copy(w.bitcast(U32).at[:, i * per_blk + t, :],
                                     wqkv.at[m * HP + i * per_blk + t],
                                     sem_qkv.at[i % 2, m * per_blk + t])
               for m, w in enumerate((wq_hbm, wk_hbm, wv_hbm)) for t in range(per_blk)]
        cps.append(pltpu.make_async_copy(
            wo_hbm.at[:, :, pl.ds(pl.multiple_of(i * 128, 128), 128)], wo.at[i],
            sem_qkv.at[i % 2, 3 * per_blk]))
        return cps

    def repack(j):
        for k in range(n_tiles):
            w = wqkv[j, k * 128:(k + 1) * 128, :]
            even = pltpu.bitcast(w << 16, F32).astype(BF16)
            odd = pltpu.bitcast(w & U32(0xFFFF0000), F32).astype(BF16)
            wqkv[j, k * 128:k * 128 + 64, :] = pltpu.bitcast(even, U32)
            wqkv[j, k * 128 + 64:(k + 1) * 128, :] = pltpu.bitcast(odd, U32)

    cp_x0.start()
    cp_w1.start()

    hbuf[0:HALO, :] = jnp.zeros((HALO, D), F32)
    hbuf[HALO + S:, :] = jnp.zeros((HALO, D), F32)
    cp_x0.wait()
    cp_w1.wait()
    for cp in (cp_x1, cp_w2, cp_w3, cp_w4):
        cp.start()

    def b1_body(i, carry):
        r = pl.multiple_of(i * ROWS_B, ROWS_B)
        x = ax[pl.ds(r, ROWS_B), :].astype(F32)
        h = _gelu(_dot(_layernorm(x).astype(BF16), w1[...]))
        hbuf[pl.ds(pl.multiple_of(r + HALO, 8), ROWS_B), :] = h
        return carry

    b1_body(0, 0)
    cp_x1.wait()
    lax.fori_loop(1, n_blk, b1_body, 0)

    for cp in a_copies(0):
        cp.start()
    cp_w2.wait()
    cp_w3.wait()
    cp_w4.wait()

    gw = gw_ref[...].reshape(1, D).astype(F32)
    c = D // 4

    def b2_body(i, carry):
        @pl.when(i + 1 < n_blk)
        def _():
            for cp in a_copies(i + 1):
                cp.start()

        for cp in a_copies(i):
            cp.wait()
        r = pl.multiple_of(i * ROWS_B, ROWS_B)
        parts = []
        for j, shift in enumerate((-1, 1, -2, 2)):
            win = hbuf[pl.ds(r, ROWS_B + 2 * HALO), pl.ds(j * c, c)]
            parts.append(win[HALO + shift:HALO + shift + ROWS_B].astype(BF16))
        hs = _dot(jnp.concatenate(parts, axis=1), w2[...])
        xa = ax[pl.ds(r, ROWS_B), :].astype(F32)
        x1 = xa + hs
        ln = _layernorm(x1).astype(BF16)
        acc = x1
        todo = [m * HP + i * per_blk + t for m in range(3) for t in range(per_blk)]
        for f in range(0, F, F_CHUNK):
            if todo:
                repack(todo.pop())
            a = _gelu(_dot(ln, w3[:, f:f + F_CHUNK])).astype(BF16)
            acc = acc + _dot(a, w4[f:f + F_CHUNK, :])
        g = jax.nn.sigmoid(jnp.sum(xa * gw, axis=-1, keepdims=True))
        bres[pl.ds(r, ROWS_B), :] = (1.0 - g) * acc
        gate[pl.ds(r, ROWS_B), :] = jnp.broadcast_to(g, (ROWS_B, 128))
        assert not todo
        return carry

    lax.fori_loop(0, n_blk, b2_body, 0)

    def head_weight(i, h):
        j = i * HP + h // 2
        off = (h % 2) * 64
        w = jnp.concatenate(
            [wqkv[j, k * 128 + off:k * 128 + off + 64, :] for k in range(n_tiles)], axis=0)
        return pltpu.bitcast(w, BF16)

    row = lax.broadcasted_iota(jnp.int32, (L, L), 0)
    col = lax.broadcasted_iota(jnp.int32, (L, L), 1)
    mask = (row < M) | (row >= col)

    hseg[0:M, :] = mem0_ref[0].astype(F32)

    def out_copy(r):
        return pltpu.make_async_copy(outbuf.at[pl.ds(r, seg)], out_hbm.at[0, pl.ds(r, seg)],
                                     sem_out)

    def seg_body(s, carry):
        r = pl.multiple_of(s * seg, seg)
        hseg[M:L, :] = ax[pl.ds(r, seg), :].astype(F32)
        qkv = {}
        probs = {}

        def project(h):
            hh = hseg[...]
            qkv[h] = [_dot(hh, head_weight(i, h)) for i in range(3)]

        def scores(h):
            q, k, _ = qkv[h]
            sc = jnp.where(mask, _dot_nt(q, k) * scale, -1000000000.0)
            e = jnp.exp(sc - jnp.max(sc, axis=-1, keepdims=True))
            probs[h] = e / jnp.sum(e, axis=-1, keepdims=True)

        def values(h):
            obuf[:, h * E:(h + 1) * E] = _dot(probs.pop(h), qkv.pop(h)[2])

        def out_part(h0, h1, n):
            w = wo[n, h0:h1].reshape((h1 - h0) * E, 128)
            return _dot(obuf[:, h0 * E:h1 * E], w)

        for h in range(H):
            project(h)
            if h >= 1:
                scores(h - 1)
            if h >= 3:
                values(h - 3)
        half = H // 2
        tail = {0: [(scores, H - 1), (values, H - 3)], 2: [(values, H - 2)], 3: [(values, H - 1)]}
        for n in range(n_tiles):
            oacc[:, n * 128:(n + 1) * 128] = out_part(0, half, n)
            for fn, h in tail.get(n, ()):
                fn(h)
        g = gate[pl.ds(r, seg), :]
        for n in range(n_tiles):
            cols = slice(n * 128, (n + 1) * 128)
            o = oacc[:, cols] + out_part(half, H, n)
            hseg[0:M, cols] = o[0:M]
            outbuf[pl.ds(r, seg), cols] = (g * o[M:L] + bres[pl.ds(r, seg), cols]).astype(BF16)
        out_copy(r).start()
        return carry

    lax.fori_loop(0, n_seg, seg_body, 0)
    pltpu.make_async_copy(outbuf, out_hbm.at[0], sem_out).wait()


@functools.partial(jax.jit, static_argnames=("A_seg_len",))
def pallas_gated_mix__memory_aug_recurrent_mem_tr__mixer_s_mlp__prompt_kernel(
    A_x: jax.Array,
    A_mem0: jax.Array,
    A_Wq: jax.Array,
    A_Wk: jax.Array,
    A_Wv: jax.Array,
    A_Wo: jax.Array,
    A_seg_len: int,
    B_x: jax.Array,
    B_w1: jax.Array,
    B_w2: jax.Array,
    B_w3: jax.Array,
    B_w4: jax.Array,
    gate_w: jax.Array,
):
    _, S, D = A_x.shape
    _, H, E = A_Wq.shape
    M = A_mem0.shape[1]
    F = B_w3.shape[1]
    seg = int(A_seg_len)
    hbm = pl.BlockSpec(memory_space=pl.ANY)
    vmem = pl.BlockSpec(memory_space=pltpu.VMEM)
    return pl.pallas_call(
        functools.partial(_kernel, seg=seg),
        out_shape=jax.ShapeDtypeStruct(A_x.shape, A_x.dtype),
        in_specs=[hbm, vmem, hbm, hbm, hbm, hbm, hbm, hbm, hbm, hbm, vmem],
        out_specs=hbm,
        scratch_shapes=[
            pltpu.VMEM((3 * H // 2, D, E), U32),
            pltpu.VMEM((D // 128, H, E, 128), BF16),
            pltpu.VMEM((D, D), BF16),
            pltpu.VMEM((D, D), BF16),
            pltpu.VMEM((D, F), BF16),
            pltpu.VMEM((F, D), BF16),
            pltpu.VMEM((S, D), BF16),
            pltpu.VMEM((S + 2 * HALO, D), F32),
            pltpu.VMEM((S, D), F32),
            pltpu.VMEM((S, 128), F32),
            pltpu.VMEM((M + seg, D), F32),
            pltpu.VMEM((M + seg, H * E), F32),
            pltpu.VMEM((M + seg, D), F32),
            pltpu.VMEM((S, D), BF16),
            pltpu.SemaphoreType.DMA((6,)),
            pltpu.SemaphoreType.DMA((2, 3 * (H // 2) * ROWS_B // S + 1)),
            pltpu.SemaphoreType.DMA(()),
        ],
        compiler_params=pltpu.CompilerParams(vmem_limit_bytes=120 * 1024 * 1024),
    )(A_x, A_mem0, A_Wq, A_Wk, A_Wv, A_Wo, B_w1, B_w2, B_w3, B_w4, gate_w)
```

```python
import functools

import jax
import jax.numpy as jnp
from jax import lax
import jax.experimental.pallas as pl
import jax.experimental.pallas.tpu as pltpu

F32 = jnp.float32
BF16 = jnp.bfloat16
U32 = jnp.uint32

ROWS_X = 256
MARKS = (0, 1, 2, 3, 4, 5, 5, 6)
F_CHUNK = 1792
HALO = 8


def _dot(a, b):
    return lax.dot_general(a, b, (((1,), (0,)), ((), ())), preferred_element_type=F32)


def _dot_nt(a, b):
    return lax.dot_general(a, b, (((1,), (1,)), ((), ())), preferred_element_type=F32)


def _layernorm(x, eps=1e-05):
    m = jnp.mean(x, axis=-1, keepdims=True)
    c = x - m
    v = jnp.mean(c * c, axis=-1, keepdims=True)
    return c * lax.rsqrt(v + eps)


def _gelu(x):
    return jax.nn.gelu(x, approximate=True)


def _kernel(ax_hbm, mem0_ref, wq_hbm, wk_hbm, wv_hbm, wo_hbm, w1_hbm, w2_hbm,
            w3_hbm, w4_hbm, gw_ref, out_hbm,
            wqkv, wo, w1, w2, w3, w4, ax, hbuf, bres, gate, hseg, obuf, oacc, outbuf, lhs0, lhs1,
            sem_in, sem_qkv, sem_wo, sem_out, *, seg):
    S, D = ax.shape
    H, E = wq_hbm.shape[1], wq_hbm.shape[2]
    HP = H // 2
    M = mem0_ref.shape[1]
    L = M + seg
    F = w3.shape[1]
    n_seg = S // seg
    n_tiles = D // 128
    scale = E ** (-0.5)

    def copy(src, dst, i):
        return pltpu.make_async_copy(src, dst, sem_in.at[i])

    n_x = S // ROWS_X
    cp_x = [copy(ax_hbm.at[0, pl.ds(i * ROWS_X, ROWS_X)], ax.at[pl.ds(i * ROWS_X, ROWS_X)], i)
            for i in range(n_x)]
    w1_cols = [pl.ds(i * (D // 4), D // 4) for i in range(4)]
    cp_w1 = [copy(w1_hbm.at[:, cs], w1.at[:, cs], n_x + i) for i, cs in enumerate(w1_cols)]
    cp_w2 = copy(w2_hbm, w2, n_x + 4)
    cp_w3 = copy(w3_hbm, w3, n_x + 5)
    cp_w4 = copy(w4_hbm, w4, n_x + 6)

    n_blk = S // ROWS_X
    per_blk = HP // n_blk

    def qkv_copies(i):
        return [pltpu.make_async_copy(w.bitcast(U32).at[:, i * per_blk + t, :],
                                      wqkv.at[m * HP + i * per_blk + t],
                                      sem_qkv.at[m * HP + i * per_blk + t])
                for m, w in enumerate((wq_hbm, wk_hbm, wv_hbm)) for t in range(per_blk)]

    def wo_copy(n):
        cols = pl.ds(pl.multiple_of(n * 128, 128), 128)
        return pltpu.make_async_copy(wo_hbm.at[:, :, cols], wo.at[n], sem_wo.at[n])

    for cp in [cp_x[0]] + cp_w1 + cp_x[1:] + [cp_w2, cp_w3, cp_w4]:
        cp.start()

    def after(dep, x):
        always = (pltpu.bitcast(dep, U32) | U32(1)) != U32(0)
        reps = (x.shape[0] // dep.shape[0], x.shape[1] // dep.shape[1])
        return jnp.where(jnp.tile(always, reps), x, jnp.zeros_like(x))

    def spread(deps, x):
        n = x.shape[0] // len(deps)
        return jnp.concatenate([after(d, x[i * n:(i + 1) * n]) for i, d in enumerate(deps)], axis=0)

    def marks(y):
        return [y[0:8, n * 128:(n + 1) * 128] for n in MARKS]

    R = ROWS_X
    lhs = (lhs0, lhs1)
    hbuf[0:HALO, :] = jnp.zeros((HALO, D), F32)
    hbuf[HALO + S:, :] = jnp.zeros((HALO, D), F32)
    gw = gw_ref[...].reshape(1, D).astype(F32)

    def rows(i, offset=0, extra=0):
        return pl.ds(pl.multiple_of(i * R + offset, 8), R + extra)

    def prepare1(i, slot, deps):
        x = ax[rows(i), :].astype(F32)
        if deps is not None:
            x = spread(deps, x)
        g = jax.nn.sigmoid(jnp.sum(x * gw, axis=-1, keepdims=True))
        gate[rows(i), :] = jnp.broadcast_to(g, (R, 128))
        lhs[slot][...] = _layernorm(x).astype(BF16)

    def stage1(i, slot):
        pre = _dot(lhs[slot][...], w1[...])
        hbuf[rows(i, HALO), :] = _gelu(pre)
        prepare1(jnp.minimum(i + 1, n_x - 1), 1 - slot, marks(pre))

    def pairs(stage):
        def body(j, carry):
            stage(2 * j, 0)
            stage(2 * j + 1, 1)
            return carry
        return body

    cp_x[0].wait()
    prepare1(0, 0, None)
    for cp, cs in zip(cp_w1, w1_cols):
        cp.wait()
        if cp is cp_w1[-1]:
            cp_x[1].wait()
        pre = _dot(lhs0[...], w1[:, cs])
        hbuf[HALO:HALO + R, cs] = _gelu(pre)
    prepare1(1, 1, [pre[0:8, 0:128]])
    cp_x[2].wait()
    stage1(1, 1)
    for cp in cp_x[3:]:
        cp.wait()
    lax.fori_loop(1, n_x // 2, pairs(stage1), 0)

    c = D // 4

    def prepare2(i, slot, deps):
        for j, shift in enumerate((-1, 1, -2, 2)):
            win = hbuf[rows(i, 0, 2 * HALO), j * c:(j + 1) * c]
            part = win[HALO + shift:HALO + shift + R]
            if deps is not None:
                part = spread(deps, part)
            lhs[slot][:, j * c:(j + 1) * c] = part.astype(BF16)

    def stage2(i, slot):
        hs = _dot(lhs[slot][...], w2[...])
        x1 = ax[rows(i), :].astype(F32) + hs
        bres[rows(i), :] = x1
        outbuf[rows(i), :] = _layernorm(x1).astype(BF16)
        prepare2(jnp.minimum(i + 1, n_x - 1), 1 - slot, marks(hs))

    cp_w2.wait()
    for cp in qkv_copies(0):
        cp.start()
    prepare2(0, 0, None)
    lax.fori_loop(0, n_x // 2, pairs(stage2), 0)

    def repack(j, k, dep):
        w = after(dep, wqkv[j, k * 128:(k + 1) * 128, :])
        even = pltpu.bitcast(w << 16, F32).astype(BF16)
        odd = pltpu.bitcast(w & U32(0xFFFF0000), F32).astype(BF16)
        wqkv[j, k * 128:k * 128 + 64, :] = pltpu.bitcast(even, U32)
        wqkv[j, k * 128 + 64:(k + 1) * 128, :] = pltpu.bitcast(odd, U32)

    def mlp_body(i, carry):
        @pl.when(i + 1 < n_blk)
        def _():
            for cp in qkv_copies(i + 1):
                cp.start()

        wo_copy(i).start()
        for cp in qkv_copies(i):
            cp.wait()
        ln = outbuf[rows(i), :]
        acc = bres[rows(i), :]
        todo = [(m * HP + i * per_blk + t, k)
                for m in range(3) for t in range(per_blk) for k in range(n_tiles)]
        n_dep = -(-len(todo) // (F // F_CHUNK))
        for f in range(0, F, F_CHUNK):
            pre = _dot(ln, w3[:, f:f + F_CHUNK])
            for u in range(n_dep):
                if todo:
                    r, k = u * 32 % ROWS_X, u % (F_CHUNK // 128)
                    repack(*todo.pop(), pre[r:r + 8, k * 128:(k + 1) * 128])
            a = _gelu(pre).astype(BF16)
            acc = acc + _dot(a, w4[f:f + F_CHUNK, :])
        bres[rows(i), :] = (1.0 - jnp.tile(gate[rows(i), :], (1, n_tiles))) * acc
        assert not todo
        return carry

    cp_w3.wait()
    cp_w4.wait()
    lax.fori_loop(0, n_blk, mlp_body, 0)
    for n in range(n_tiles):
        wo_copy(n).wait()

    def head_weight(i, h):
        j = i * HP + h // 2
        off = (h % 2) * 64
        w = jnp.concatenate(
            [wqkv[j, k * 128 + off:k * 128 + off + 64, :] for k in range(n_tiles)], axis=0)
        return pltpu.bitcast(w, BF16)

    row = lax.broadcasted_iota(jnp.int32, (L, L), 0)
    col = lax.broadcasted_iota(jnp.int32, (L, L), 1)
    mask = (row < M) | (row >= col)

    hseg[0:M, :] = mem0_ref[0].astype(F32)

    def out_copy(r):
        return pltpu.make_async_copy(outbuf.at[pl.ds(r, seg)], out_hbm.at[0, pl.ds(r, seg)],
                                     sem_out)

    def seg_body(s, carry):
        r = pl.multiple_of(s * seg, seg)
        hseg[M:L, :] = ax[pl.ds(r, seg), :].astype(F32)
        qkv = {}
        probs = {}

        def project(h):
            hh = hseg[...]
            qkv[h] = [_dot(hh, head_weight(i, h)) for i in range(3)]

        def scores(h):
            q, k, _ = qkv[h]
            sc = jnp.where(mask, _dot_nt(q, k) * scale, -1000000000.0)
            e = jnp.exp(sc - jnp.max(sc, axis=-1, keepdims=True))
            probs[h] = e / jnp.sum(e, axis=-1, keepdims=True)

        def values(h):
            obuf[:, h * E:(h + 1) * E] = _dot(probs.pop(h), qkv.pop(h)[2])

        def out_part(h0, h1, n):
            w = wo[n, h0:h1].reshape((h1 - h0) * E, 128)
            return _dot(obuf[:, h0 * E:h1 * E], w)

        for h in range(H):
            project(h)
            if h >= 1:
                scores(h - 1)
            if h >= 3:
                values(h - 3)
        half = H // 2
        tail = {0: [(scores, H - 1), (values, H - 3)], 2: [(values, H - 2)], 3: [(values, H - 1)]}
        for n in range(n_tiles):
            oacc[:, n * 128:(n + 1) * 128] = out_part(0, half, n)
            for fn, h in tail.get(n, ()):
                fn(h)
        g = gate[pl.ds(r, seg), :]
        for n in range(n_tiles):
            cols = slice(n * 128, (n + 1) * 128)
            o = oacc[:, cols] + out_part(half, H, n)
            hseg[0:M, cols] = o[0:M]
            outbuf[pl.ds(r, seg), cols] = (g * o[M:L] + bres[pl.ds(r, seg), cols]).astype(BF16)
        out_copy(r).start()
        return carry

    lax.fori_loop(0, n_seg, seg_body, 0)
    pltpu.make_async_copy(outbuf, out_hbm.at[0], sem_out).wait()


@functools.partial(jax.jit, static_argnames=("A_seg_len",))
def pallas_gated_mix__memory_aug_recurrent_mem_tr__mixer_s_mlp__prompt_kernel(
    A_x: jax.Array,
    A_mem0: jax.Array,
    A_Wq: jax.Array,
    A_Wk: jax.Array,
    A_Wv: jax.Array,
    A_Wo: jax.Array,
    A_seg_len: int,
    B_x: jax.Array,
    B_w1: jax.Array,
    B_w2: jax.Array,
    B_w3: jax.Array,
    B_w4: jax.Array,
    gate_w: jax.Array,
):
    _, S, D = A_x.shape
    _, H, E = A_Wq.shape
    M = A_mem0.shape[1]
    F = B_w3.shape[1]
    seg = int(A_seg_len)
    hbm = pl.BlockSpec(memory_space=pl.ANY)
    vmem = pl.BlockSpec(memory_space=pltpu.VMEM)
    return pl.pallas_call(
        functools.partial(_kernel, seg=seg),
        out_shape=jax.ShapeDtypeStruct(A_x.shape, A_x.dtype),
        in_specs=[hbm, vmem, hbm, hbm, hbm, hbm, hbm, hbm, hbm, hbm, vmem],
        out_specs=hbm,
        scratch_shapes=[
            pltpu.VMEM((3 * H // 2, D, E), U32),
            pltpu.VMEM((D // 128, H, E, 128), BF16),
            pltpu.VMEM((D, D), BF16),
            pltpu.VMEM((D, D), BF16),
            pltpu.VMEM((D, F), BF16),
            pltpu.VMEM((F, D), BF16),
            pltpu.VMEM((S, D), BF16),
            pltpu.VMEM((S + 2 * HALO, D), F32),
            pltpu.VMEM((S, D), F32),
            pltpu.VMEM((S, 128), F32),
            pltpu.VMEM((M + seg, D), F32),
            pltpu.VMEM((M + seg, H * E), F32),
            pltpu.VMEM((M + seg, D), F32),
            pltpu.VMEM((S, D), BF16),
            pltpu.VMEM((ROWS_X, D), BF16),
            pltpu.VMEM((ROWS_X, D), BF16),
            pltpu.SemaphoreType.DMA((S // ROWS_X + 7,)),
            pltpu.SemaphoreType.DMA((3 * H // 2,)),
            pltpu.SemaphoreType.DMA((D // 128,)),
            pltpu.SemaphoreType.DMA(()),
        ],
        compiler_params=pltpu.CompilerParams(vmem_limit_bytes=120 * 1024 * 1024),
    )(A_x, A_mem0, A_Wq, A_Wk, A_Wv, A_Wo, B_w1, B_w2, B_w3, B_w4, gate_w)
```

```python
import functools

import jax
import jax.numpy as jnp
from jax import lax
import jax.experimental.pallas as pl
import jax.experimental.pallas.tpu as pltpu

F32 = jnp.float32
BF16 = jnp.bfloat16
U32 = jnp.uint32

ROWS_X = 256
MARKS = (0, 1, 2, 3, 4, 5, 5, 6)
F_CHUNK = 1792
SEG_UNROLL = 2
HALO = 8


def _dot(a, b):
    return lax.dot_general(a, b, (((1,), (0,)), ((), ())), preferred_element_type=F32)


def _dot_nt(a, b):
    return lax.dot_general(a, b, (((1,), (1,)), ((), ())), preferred_element_type=F32)


def _layernorm(x, eps=1e-05):
    m = jnp.mean(x, axis=-1, keepdims=True)
    c = x - m
    v = jnp.mean(c * c, axis=-1, keepdims=True)
    return c * lax.rsqrt(v + eps)


def _gelu(x):
    return jax.nn.gelu(x, approximate=True)


def _kernel(ax_hbm, mem0_ref, wq_hbm, wk_hbm, wv_hbm, wo_hbm, w1_hbm, w2_hbm,
            w3_hbm, w4_hbm, gw_ref, out_hbm,
            wqkv, wo, w1, w2, w3, w4, ax, hbuf, bres, gate, hseg, obuf, oacc, outbuf, lhs0, lhs1,
            sem_in, sem_qkv, sem_wo, sem_out, *, seg):
    S, D = ax.shape
    H, E = wq_hbm.shape[1], wq_hbm.shape[2]
    HP = H // 2
    M = mem0_ref.shape[1]
    L = M + seg
    F = w3.shape[1]
    n_seg = S // seg
    n_tiles = D // 128
    scale = E ** (-0.5)

    def copy(src, dst, i):
        return pltpu.make_async_copy(src, dst, sem_in.at[i])

    n_x = S // ROWS_X
    cp_x = [copy(ax_hbm.at[0, pl.ds(i * ROWS_X, ROWS_X)], ax.at[pl.ds(i * ROWS_X, ROWS_X)], i)
            for i in range(n_x)]
    w1_cols = [pl.ds(i * (D // 4), D // 4) for i in range(4)]
    cp_w1 = [copy(w1_hbm.at[:, cs], w1.at[:, cs], n_x + i) for i, cs in enumerate(w1_cols)]
    cp_w2 = copy(w2_hbm, w2, n_x + 4)
    cp_w3 = copy(w3_hbm, w3, n_x + 5)
    cp_w4 = copy(w4_hbm, w4, n_x + 6)

    n_blk = S // ROWS_X
    per_blk = HP // n_blk

    def qkv_copies(i):
        return [pltpu.make_async_copy(w.bitcast(U32).at[:, i * per_blk + t, :],
                                      wqkv.at[m * HP + i * per_blk + t],
                                      sem_qkv.at[m * HP + i * per_blk + t])
                for m, w in enumerate((wq_hbm, wk_hbm, wv_hbm)) for t in range(per_blk)]

    def wo_copy(n):
        cols = pl.ds(pl.multiple_of(n * 128, 128), 128)
        return pltpu.make_async_copy(wo_hbm.at[:, :, cols], wo.at[n], sem_wo.at[n])

    for cp in [cp_x[0]] + cp_w1 + cp_x[1:] + [cp_w2, cp_w3, cp_w4]:
        cp.start()

    def after(dep, x):
        always = (pltpu.bitcast(dep, U32) | U32(1)) != U32(0)
        reps = (x.shape[0] // dep.shape[0], x.shape[1] // dep.shape[1])
        return jnp.where(jnp.tile(always, reps), x, jnp.zeros_like(x))

    def spread(deps, x):
        n = x.shape[0] // len(deps)
        return jnp.concatenate([after(d, x[i * n:(i + 1) * n]) for i, d in enumerate(deps)], axis=0)

    def marks(y):
        return [y[0:8, n * 128:(n + 1) * 128] for n in MARKS]

    R = ROWS_X
    lhs = (lhs0, lhs1)
    hbuf[0:HALO, :] = jnp.zeros((HALO, D), F32)
    hbuf[HALO + S:, :] = jnp.zeros((HALO, D), F32)
    gw = gw_ref[...].reshape(1, D).astype(F32)

    def rows(i, offset=0, extra=0):
        return pl.ds(pl.multiple_of(i * R + offset, 8), R + extra)

    def prepare1(i, slot, deps):
        x = ax[rows(i), :].astype(F32)
        if deps is not None:
            x = spread(deps, x)
        g = jax.nn.sigmoid(jnp.sum(x * gw, axis=-1, keepdims=True))
        gate[rows(i), :] = jnp.broadcast_to(g, (R, 128))
        lhs[slot][...] = _layernorm(x).astype(BF16)

    def stage1(i, slot):
        pre = _dot(lhs[slot][...], w1[...])
        hbuf[rows(i, HALO), :] = _gelu(pre)
        prepare1(jnp.minimum(i + 1, n_x - 1), 1 - slot, marks(pre))

    def pairs(stage):
        def body(j, carry):
            stage(2 * j, 0)
            stage(2 * j + 1, 1)
            return carry
        return body

    cp_x[0].wait()
    prepare1(0, 0, None)
    for cp, cs in zip(cp_w1, w1_cols):
        cp.wait()
        if cp is cp_w1[-1]:
            cp_x[1].wait()
        pre = _dot(lhs0[...], w1[:, cs])
        hbuf[HALO:HALO + R, cs] = _gelu(pre)
    prepare1(1, 1, [pre[0:8, 0:128]])
    cp_x[2].wait()
    stage1(1, 1)
    for cp in cp_x[3:]:
        cp.wait()
    lax.fori_loop(1, n_x // 2, pairs(stage1), 0)

    c = D // 4

    def prepare2(i, slot, deps):
        for j, shift in enumerate((-1, 1, -2, 2)):
            win = hbuf[rows(i, 0, 2 * HALO), j * c:(j + 1) * c]
            part = win[HALO + shift:HALO + shift + R]
            if deps is not None:
                part = spread(deps, part)
            lhs[slot][:, j * c:(j + 1) * c] = part.astype(BF16)

    def stage2(i, slot):
        hs = _dot(lhs[slot][...], w2[...])
        x1 = ax[rows(i), :].astype(F32) + hs
        bres[rows(i), :] = x1
        outbuf[rows(i), :] = _layernorm(x1).astype(BF16)
        prepare2(jnp.minimum(i + 1, n_x - 1), 1 - slot, marks(hs))

    cp_w2.wait()
    for cp in qkv_copies(0) + qkv_copies(1):
        cp.start()
    prepare2(0, 0, None)
    lax.fori_loop(0, n_x // 2, pairs(stage2), 0)

    def repack(j, k, dep):
        w = after(dep, wqkv[j, k * 128:(k + 1) * 128, :])
        even = pltpu.bitcast(w << 16, F32).astype(BF16)
        odd = pltpu.bitcast(w & U32(0xFFFF0000), F32).astype(BF16)
        wqkv[j, k * 128:k * 128 + 64, :] = pltpu.bitcast(even, U32)
        wqkv[j, k * 128 + 64:(k + 1) * 128, :] = pltpu.bitcast(odd, U32)

    def mlp_body(i, carry):
        for cp in qkv_copies(i):
            cp.wait()
        ln = outbuf[rows(i), :]
        acc = bres[rows(i), :]
        todo = [(m * HP + i * per_blk + t, k)
                for m in range(3) for t in range(per_blk) for k in range(n_tiles)]
        n_dep = -(-len(todo) // (F // F_CHUNK))
        for f in range(0, F, F_CHUNK):
            pre = _dot(ln, w3[:, f:f + F_CHUNK])
            for u in range(n_dep):
                if todo:
                    r, k = u * 32 % ROWS_X, u % (F_CHUNK // 128)
                    repack(*todo.pop(), pre[r:r + 8, k * 128:(k + 1) * 128])
            a = _gelu(pre).astype(BF16)
            acc = acc + _dot(a, w4[f:f + F_CHUNK, :])
        bres[rows(i), :] = (1.0 - jnp.tile(gate[rows(i), :], (1, n_tiles))) * acc
        assert not todo
        wo_copy(i).start()

        @pl.when(i + 2 < n_blk)
        def _():
            for cp in qkv_copies(i + 2):
                cp.start()

        return carry

    cp_w3.wait()
    cp_w4.wait()
    lax.fori_loop(0, n_blk, mlp_body, 0)
    for n in range(n_tiles):
        wo_copy(n).wait()

    def head_weight(i, h):
        j = i * HP + h // 2
        off = (h % 2) * 64
        w = jnp.concatenate(
            [wqkv[j, k * 128 + off:k * 128 + off + 64, :] for k in range(n_tiles)], axis=0)
        return pltpu.bitcast(w, BF16)

    row = lax.broadcasted_iota(jnp.int32, (L, L), 0)
    col = lax.broadcasted_iota(jnp.int32, (L, L), 1)
    mask = (row < M) | (row >= col)

    hseg[0:M, :] = mem0_ref[0].astype(F32)

    def out_copy(r):
        return pltpu.make_async_copy(outbuf.at[pl.ds(r, seg)], out_hbm.at[0, pl.ds(r, seg)],
                                     sem_out)

    def seg_body(s, carry):
        r = pl.multiple_of(s * seg, seg)
        hseg[M:L, :] = ax[pl.ds(r, seg), :].astype(F32)
        qkv = {}
        probs = {}

        def project(h):
            hh = hseg[...]
            ws = [head_weight(i, h) for i in range(3)]
            if h == 0:
                k = D // 2
                part = [_dot(hh[:, :k], w[:k]) for w in ws]
                oacc[:, 0:3 * E] = jnp.concatenate(part, axis=1)
                qkv[h] = [oacc[:, i * E:(i + 1) * E] + _dot(hh[:, k:], w[k:]) for i, w in enumerate(ws)]
            else:
                qkv[h] = [_dot(hh, w) for w in ws]

        def scores(h):
            q, k, _ = qkv[h]
            sc = jnp.where(mask, _dot_nt(q, k) * scale, -1000000000.0)
            e = jnp.exp(sc - jnp.max(sc, axis=-1, keepdims=True))
            probs[h] = e / jnp.sum(e, axis=-1, keepdims=True)

        def values(h):
            obuf[:, h * E:(h + 1) * E] = _dot(probs.pop(h), qkv.pop(h)[2])

        def out_part(h0, h1, n):
            w = wo[n, h0:h1].reshape((h1 - h0) * E, 128)
            return _dot(obuf[:, h0 * E:h1 * E], w)

        for h in range(H):
            project(h)
            if h >= 1:
                scores(h - 1)
            if h >= 3:
                values(h - 3)
        half = H // 2
        tail = {0: [(scores, H - 1), (values, H - 3)], 2: [(values, H - 2)], 3: [(values, H - 1)]}
        for n in range(n_tiles):
            oacc[:, n * 128:(n + 1) * 128] = out_part(0, half, n)
            for fn, h in tail.get(n, ()):
                fn(h)
        g = gate[pl.ds(r, seg), :]
        for n in range(n_tiles):
            cols = slice(n * 128, (n + 1) * 128)
            o = oacc[:, cols] + out_part(half, H, n)
            hseg[0:M, cols] = o[0:M]
            outbuf[pl.ds(r, seg), cols] = (g * o[M:L] + bres[pl.ds(r, seg), cols]).astype(BF16)
        out_copy(r).start()
        return carry

    lax.fori_loop(0, n_seg, seg_body, 0, unroll=SEG_UNROLL)
    pltpu.make_async_copy(outbuf, out_hbm.at[0], sem_out).wait()


@functools.partial(jax.jit, static_argnames=("A_seg_len",))
def pallas_gated_mix__memory_aug_recurrent_mem_tr__mixer_s_mlp__prompt_kernel(
    A_x: jax.Array,
    A_mem0: jax.Array,
    A_Wq: jax.Array,
    A_Wk: jax.Array,
    A_Wv: jax.Array,
    A_Wo: jax.Array,
    A_seg_len: int,
    B_x: jax.Array,
    B_w1: jax.Array,
    B_w2: jax.Array,
    B_w3: jax.Array,
    B_w4: jax.Array,
    gate_w: jax.Array,
):
    _, S, D = A_x.shape
    _, H, E = A_Wq.shape
    M = A_mem0.shape[1]
    F = B_w3.shape[1]
    seg = int(A_seg_len)
    hbm = pl.BlockSpec(memory_space=pl.ANY)
    vmem = pl.BlockSpec(memory_space=pltpu.VMEM)
    return pl.pallas_call(
        functools.partial(_kernel, seg=seg),
        out_shape=jax.ShapeDtypeStruct(A_x.shape, A_x.dtype),
        in_specs=[hbm, vmem, hbm, hbm, hbm, hbm, hbm, hbm, hbm, hbm, vmem],
        out_specs=hbm,
        scratch_shapes=[
            pltpu.VMEM((3 * H // 2, D, E), U32),
            pltpu.VMEM((D // 128, H, E, 128), BF16),
            pltpu.VMEM((D, D), BF16),
            pltpu.VMEM((D, D), BF16),
            pltpu.VMEM((D, F), BF16),
            pltpu.VMEM((F, D), BF16),
            pltpu.VMEM((S, D), BF16),
            pltpu.VMEM((S + 2 * HALO, D), F32),
            pltpu.VMEM((S, D), F32),
            pltpu.VMEM((S, 128), F32),
            pltpu.VMEM((M + seg, D), F32),
            pltpu.VMEM((M + seg, H * E), F32),
            pltpu.VMEM((M + seg, D), F32),
            pltpu.VMEM((S, D), BF16),
            pltpu.VMEM((ROWS_X, D), BF16),
            pltpu.VMEM((ROWS_X, D), BF16),
            pltpu.SemaphoreType.DMA((S // ROWS_X + 7,)),
            pltpu.SemaphoreType.DMA((3 * H // 2,)),
            pltpu.SemaphoreType.DMA((D // 128,)),
            pltpu.SemaphoreType.DMA(()),
        ],
        compiler_params=pltpu.CompilerParams(vmem_limit_bytes=120 * 1024 * 1024, disable_bounds_checks=True),
    )(A_x, A_mem0, A_Wq, A_Wk, A_Wv, A_Wo, B_w1, B_w2, B_w3, B_w4, gate_w)
```

```python
import functools

import jax
import jax.numpy as jnp
from jax import lax
import jax.experimental.pallas as pl
import jax.experimental.pallas.tpu as pltpu

F32 = jnp.float32
BF16 = jnp.bfloat16
U32 = jnp.uint32

ROWS_X = 256
W1_SPLIT = (0, 512, 1024)
X1_AT = 1
GROUP_2 = 4
MARKS = (0, 1, 2, 3, 4, 5, 6, 6)
SEG_UNROLL = 2
HALO = 8


def _dot(a, b):
    return lax.dot_general(a, b, (((1,), (0,)), ((), ())), preferred_element_type=F32)


def _dot_nt(a, b):
    return lax.dot_general(a, b, (((1,), (1,)), ((), ())), preferred_element_type=F32)


def _layernorm(x, eps=1e-05):
    m = jnp.mean(x, axis=-1, keepdims=True)
    c = x - m
    v = jnp.mean(c * c, axis=-1, keepdims=True)
    return c * lax.rsqrt(v + eps)


def _gelu(x):
    return jax.nn.gelu(x, approximate=True)


def _kernel(ax_hbm, mem0_hbm, wq_hbm, wk_hbm, wv_hbm, wo_hbm, w1_hbm, w2_hbm,
            w3_hbm, w4_hbm, gw_hbm, out_hbm,
            wqkv, wo, w1, w2, w3, w4, ax, hbuf, bres, gate, hseg, obuf, oacc, outbuf, lhs0, lhs1,
            mem0_ref, gw_ref,
            sem_in, sem_qkv, sem_wo, sem_out, *, seg):
    S, D = ax.shape
    H, E = wq_hbm.shape[1], wq_hbm.shape[2]
    HP = H // 2
    M = mem0_ref.shape[1]
    L = M + seg
    F = w3.shape[1]
    n_seg = S // seg
    n_tiles = D // 128
    scale = E ** (-0.5)

    def copy(src, dst, i):
        return pltpu.make_async_copy(src, dst, sem_in.at[i])

    R = ROWS_X
    n_x = S // R
    x_rows = [pl.ds(0, R), pl.ds(R, R)] + [pl.ds(i * R, 2 * R) for i in range(2, n_x, 2)]
    cp_x = [copy(ax_hbm.at[0, rs], ax.at[rs], i) for i, rs in enumerate(x_rows)]
    w1_rows = [slice(r0, r1) for r0, r1 in zip(W1_SPLIT, W1_SPLIT[1:])]
    cp_w1 = [copy(w1_hbm.at[rs], w1.at[rs], n_x + i) for i, rs in enumerate(w1_rows)]
    cp_w2, cp_w3, cp_w4, cp_gw, cp_mem = [
        copy(src, dst, n_x + len(w1_rows) + i) for i, (src, dst) in enumerate(
            ((w2_hbm, w2), (w3_hbm, w3), (w4_hbm, w4), (gw_hbm, gw_ref), (mem0_hbm, mem0_ref)))]

    n_blk = S // ROWS_X
    per_blk = HP // n_blk

    def qkv_copies(i):
        return [pltpu.make_async_copy(w.bitcast(U32).at[:, i * per_blk + t, :],
                                      wqkv.at[m * HP + i * per_blk + t],
                                      sem_qkv.at[m * HP + i * per_blk + t])
                for m, w in enumerate((wq_hbm, wk_hbm, wv_hbm)) for t in range(per_blk)]

    def wo_copy(n):
        cols = pl.ds(pl.multiple_of(n * 128, 128), 128)
        return pltpu.make_async_copy(wo_hbm.at[:, :, cols], wo.at[n], sem_wo.at[n])

    for cp in (cp_x[:1] + [cp_gw] + cp_w1[:X1_AT] + cp_x[1:2] + cp_w1[X1_AT:] + cp_x[2:]
               + [cp_w2, cp_mem, cp_w3, cp_w4]):
        cp.start()

    def after(dep, x):
        always = (pltpu.bitcast(dep, U32) | U32(1)) != U32(0)
        reps = (x.shape[0] // dep.shape[0], x.shape[1] // dep.shape[1])
        return jnp.where(jnp.tile(always, reps), x, jnp.zeros_like(x))

    def spread(deps, x):
        n = x.shape[0] // len(deps)
        return jnp.concatenate([after(d, x[i * n:(i + 1) * n]) for i, d in enumerate(deps)], axis=0)

    def marks(y):
        return [y[0:8, n * 128:(n + 1) * 128] for n in MARKS]

    lhs = (lhs0, lhs1)
    hbuf[:, 0:HALO, :] = jnp.zeros((n_tiles, HALO, 128), F32)
    hbuf[:, HALO + S:, :] = jnp.zeros((n_tiles, HALO, 128), F32)

    def store_h(rs, h):
        for n in range(n_tiles):
            hbuf[n, rs, :] = h[:, n * 128:(n + 1) * 128]

    def rows(i, offset=0, extra=0):
        return pl.ds(pl.multiple_of(i * R + offset, 8), R + extra)

    def prepare1(i, slot, deps):
        x = ax[rows(i), :].astype(F32)
        if deps is not None:
            x = spread(deps, x)
        gw = gw_ref[...].reshape(1, D).astype(F32)
        g = jax.nn.sigmoid(jnp.sum(x * gw, axis=-1, keepdims=True))
        gate[rows(i), :] = jnp.broadcast_to(g, (R, 128))
        lhs[slot][...] = _layernorm(x).astype(BF16)

    def stage1(i, slot):
        pre = _dot(lhs[slot][...], w1[...])
        store_h(rows(i, HALO), _gelu(pre))
        prepare1(jnp.minimum(i + 1, n_x - 1), 1 - slot, marks(pre))

    def pair1(j, carry):
        for k in range(2, n_x // 2):
            pl.when(j + 1 == k)(cp_x[k + 1].wait)
        stage1(2 * j, 0)
        stage1(2 * j + 1, 1)
        return carry

    cp_x[0].wait()
    cp_gw.wait()
    prepare1(0, 0, None)
    for i, (cp, rs) in enumerate(zip(cp_w1, w1_rows)):
        if i == X1_AT:
            cp_x[1].wait()
            prepare1(1, 1, None)
        cp.wait()
        pre = _dot(lhs0[:, rs], w1[rs, :])
        if i > 0:
            pre = bres[0:R, :] + pre
        if i < len(cp_w1) - 1:
            bres[0:R, :] = pre
    store_h(rows(0, HALO), _gelu(pre))
    cp_x[2].wait()
    stage1(1, 1)
    lax.fori_loop(1, n_x // 2, pair1, 0)

    c = D // 4

    def prepare2(i, slot, deps):
        for n in range(n_tiles):
            shift = (-1, 1, -2, 2)[n * 128 // c]
            part = hbuf[n, pl.ds(i * R + HALO + shift, R), :]
            if deps is not None:
                part = spread(deps, part)
            lhs[slot][:, n * 128:(n + 1) * 128] = part.astype(BF16)

    def stage2(i, slot):
        hs = _dot(lhs[slot][...], w2[...])
        x1 = ax[rows(i), :].astype(F32) + hs
        bres[rows(i), :] = x1
        outbuf[rows(i), :] = _layernorm(x1).astype(BF16)
        prepare2(jnp.minimum(i + 1, n_x - 1), 1 - slot, marks(hs))

    def group2(j, carry):
        for t in range(GROUP_2):
            stage2(GROUP_2 * j + t, t % 2)
        return carry

    cp_w2.wait()
    for cp in qkv_copies(0) + qkv_copies(1):
        cp.start()
    prepare2(0, 0, None)
    lax.fori_loop(0, n_x // GROUP_2, group2, 0)

    def repack(j, k, dep):
        w = after(dep, wqkv[j, k * 128:(k + 1) * 128, :])
        even = pltpu.bitcast(w << 16, F32).astype(BF16)
        odd = pltpu.bitcast(w & U32(0xFFFF0000), F32).astype(BF16)
        wqkv[j, k * 128:k * 128 + 64, :] = pltpu.bitcast(even, U32)
        wqkv[j, k * 128 + 64:(k + 1) * 128, :] = pltpu.bitcast(odd, U32)

    def mlp_body(i, carry):
        for cp in qkv_copies(i):
            cp.wait()
        pre = _dot(outbuf[rows(i), :], w3[...])
        todo = [(m * HP + i * per_blk + t, k)
                for m in range(3) for t in range(per_blk) for k in range(n_tiles)]
        for u, (j, k) in enumerate(todo):
            n, r = divmod(u * 2 * (F // 128) // len(todo), 2)
            repack(j, k, pre[r * (R // 2):r * (R // 2) + 8, n * 128:(n + 1) * 128])
        y = _dot(_gelu(pre).astype(BF16), w4[...])
        bres[rows(i), :] = (1.0 - jnp.tile(gate[rows(i), :], (1, n_tiles))) * (bres[rows(i), :] + y)
        wo_copy(i).start()

        @pl.when(i + 2 < n_blk)
        def _():
            for cp in qkv_copies(i + 2):
                cp.start()

        return carry

    cp_w3.wait()
    cp_w4.wait()
    lax.fori_loop(0, n_blk, mlp_body, 0)
    for n in range(n_tiles):
        wo_copy(n).wait()

    def head_weight(i, h):
        j = i * HP + h // 2
        off = (h % 2) * 64
        w = jnp.concatenate(
            [wqkv[j, k * 128 + off:k * 128 + off + 64, :] for k in range(n_tiles)], axis=0)
        return pltpu.bitcast(w, BF16)

    row = lax.broadcasted_iota(jnp.int32, (L, L), 0)
    col = lax.broadcasted_iota(jnp.int32, (L, L), 1)
    mask = (row < M) | (row >= col)

    cp_mem.wait()
    hseg[0:M, :] = mem0_ref[0].astype(F32)

    def out_copy(r):
        return pltpu.make_async_copy(outbuf.at[pl.ds(r, seg)], out_hbm.at[0, pl.ds(r, seg)],
                                     sem_out)

    def seg_body(s, carry):
        r = pl.multiple_of(s * seg, seg)
        hseg[M:L, :] = ax[pl.ds(r, seg), :].astype(F32)
        qkv = {}
        probs = {}

        def project(h):
            hh = hseg[...]
            ws = [head_weight(i, h) for i in range(3)]
            if h == 0:
                k = D // 2
                part = [_dot(hh[:, :k], w[:k]) for w in ws]
                oacc[:, 0:3 * E] = jnp.concatenate(part, axis=1)
                qkv[h] = [oacc[:, i * E:(i + 1) * E] + _dot(hh[:, k:], w[k:]) for i, w in enumerate(ws)]
            else:
                qkv[h] = [_dot(hh, w) for w in ws]

        def scores(h):
            q, k, _ = qkv[h]
            sc = jnp.where(mask, _dot_nt(q, k) * scale, -1000000000.0)
            e = jnp.exp(sc - jnp.max(sc, axis=-1, keepdims=True))
            probs[h] = e / jnp.sum(e, axis=-1, keepdims=True)

        def values(h):
            obuf[:, h * E:(h + 1) * E] = _dot(probs.pop(h), qkv.pop(h)[2])

        def out_part(h0, h1, n):
            w = wo[n, h0:h1].reshape((h1 - h0) * E, 128)
            return _dot(obuf[:, h0 * E:h1 * E], w)

        for h in range(H):
            project(h)
            if h >= 1:
                scores(h - 1)
            if h >= 3:
                values(h - 3)
        half = H // 2
        tail = {0: [(scores, H - 1), (values, H - 3)], 2: [(values, H - 2)], 3: [(values, H - 1)]}
        for n in range(n_tiles):
            oacc[:, n * 128:(n + 1) * 128] = out_part(0, half, n)
            for fn, h in tail.get(n, ()):
                fn(h)
        g = gate[pl.ds(r, seg), :]
        for n in range(n_tiles):
            cols = slice(n * 128, (n + 1) * 128)
            o = oacc[:, cols] + out_part(half, H, n)
            hseg[0:M, cols] = o[0:M]
            outbuf[pl.ds(r, seg), cols] = (g * o[M:L] + bres[pl.ds(r, seg), cols]).astype(BF16)
        out_copy(r).start()
        return carry

    lax.fori_loop(0, n_seg, seg_body, 0, unroll=SEG_UNROLL)
    pltpu.make_async_copy(outbuf, out_hbm.at[0], sem_out).wait()


@functools.partial(jax.jit, static_argnames=("A_seg_len",))
def pallas_gated_mix__memory_aug_recurrent_mem_tr__mixer_s_mlp__prompt_kernel(
    A_x: jax.Array,
    A_mem0: jax.Array,
    A_Wq: jax.Array,
    A_Wk: jax.Array,
    A_Wv: jax.Array,
    A_Wo: jax.Array,
    A_seg_len: int,
    B_x: jax.Array,
    B_w1: jax.Array,
    B_w2: jax.Array,
    B_w3: jax.Array,
    B_w4: jax.Array,
    gate_w: jax.Array,
):
    _, S, D = A_x.shape
    _, H, E = A_Wq.shape
    M = A_mem0.shape[1]
    F = B_w3.shape[1]
    seg = int(A_seg_len)
    hbm = pl.BlockSpec(memory_space=pl.ANY)
    return pl.pallas_call(
        functools.partial(_kernel, seg=seg),
        out_shape=jax.ShapeDtypeStruct(A_x.shape, A_x.dtype),
        in_specs=[hbm] * 11,
        out_specs=hbm,
        scratch_shapes=[
            pltpu.VMEM((3 * H // 2, D, E), U32),
            pltpu.VMEM((D // 128, H, E, 128), BF16),
            pltpu.VMEM((D, D), BF16),
            pltpu.VMEM((D, D), BF16),
            pltpu.VMEM((D, F), BF16),
            pltpu.VMEM((F, D), BF16),
            pltpu.VMEM((S, D), BF16),
            pltpu.VMEM((D // 128, S + 2 * HALO, 128), F32),
            pltpu.VMEM((S, D), F32),
            pltpu.VMEM((S, 128), F32),
            pltpu.VMEM((M + seg, D), F32),
            pltpu.VMEM((M + seg, H * E), F32),
            pltpu.VMEM((M + seg, D), F32),
            pltpu.VMEM((S, D), BF16),
            pltpu.VMEM((ROWS_X, D), BF16),
            pltpu.VMEM((ROWS_X, D), BF16),
            pltpu.VMEM(A_mem0.shape, BF16),
            pltpu.VMEM(gate_w.shape, BF16),
            pltpu.SemaphoreType.DMA((S // ROWS_X + len(W1_SPLIT) + 4,)),
            pltpu.SemaphoreType.DMA((3 * H // 2,)),
            pltpu.SemaphoreType.DMA((D // 128,)),
            pltpu.SemaphoreType.DMA(()),
        ],
        compiler_params=pltpu.CompilerParams(vmem_limit_bytes=120 * 1024 * 1024, disable_bounds_checks=True),
    )(A_x, A_mem0, A_Wq, A_Wk, A_Wv, A_Wo, B_w1, B_w2, B_w3, B_w4, gate_w)
```

```python
import functools

import jax
import jax.numpy as jnp
from jax import lax
import jax.experimental.pallas as pl
import jax.experimental.pallas.tpu as pltpu

F32 = jnp.float32
BF16 = jnp.bfloat16
U32 = jnp.uint32

ROWS_X = 256
W1_SPLIT = (0, 512, 1024)
X1_AT = 1
GROUP_2 = 4
N_MARKS = 32
MARK_END = 28
SUB = 4
SEG_UNROLL = 2
HALO = 8


def _dot(a, b):
    return lax.dot_general(a, b, (((1,), (0,)), ((), ())), preferred_element_type=F32)


def _dot_nt(a, b):
    return lax.dot_general(a, b, (((1,), (1,)), ((), ())), preferred_element_type=F32)


def _layernorm(x, eps=1e-05):
    m = jnp.mean(x, axis=-1, keepdims=True)
    c = x - m
    v = jnp.mean(c * c, axis=-1, keepdims=True)
    return c * lax.rsqrt(v + eps)


def _gelu(x):
    return jax.nn.gelu(x, approximate=True)


def _kernel(ax_hbm, mem0_hbm, wq_hbm, wk_hbm, wv_hbm, wo_hbm, w1_hbm, w2_hbm,
            w3_hbm, w4_hbm, gw_hbm, out_hbm,
            wqkv, wo, w1, w2, w3, w4, ax, hbuf, bres, gate, hseg, obuf, oacc, outbuf, lhs0, lhs1,
            mem0_ref, gw_ref,
            sem_in, sem_qkv, sem_wo, sem_out, *, seg):
    S, D = ax.shape
    H, E = wq_hbm.shape[1], wq_hbm.shape[2]
    HP = H // 2
    M = mem0_ref.shape[1]
    L = M + seg
    F = w3.shape[1]
    n_seg = S // seg
    n_tiles = D // 128
    scale = E ** (-0.5)

    def copy(src, dst, i):
        return pltpu.make_async_copy(src, dst, sem_in.at[i])

    R = ROWS_X
    n_x = S // R
    x_rows = [pl.ds(0, R), pl.ds(R, R)] + [pl.ds(i * R, 2 * R) for i in range(2, n_x, 2)]
    cp_x = [copy(ax_hbm.at[0, rs], ax.at[rs], i) for i, rs in enumerate(x_rows)]
    w1_rows = [slice(r0, r1) for r0, r1 in zip(W1_SPLIT, W1_SPLIT[1:])]
    cp_w1 = [copy(w1_hbm.at[rs], w1.at[rs], n_x + i) for i, rs in enumerate(w1_rows)]
    cp_w2, cp_w3, cp_w4, cp_gw, cp_mem = [
        copy(src, dst, n_x + len(w1_rows) + i) for i, (src, dst) in enumerate(
            ((w2_hbm, w2), (w3_hbm, w3), (w4_hbm, w4), (gw_hbm, gw_ref), (mem0_hbm, mem0_ref)))]

    n_blk = S // ROWS_X
    per_blk = HP // n_blk

    def qkv_copies(i):
        return [pltpu.make_async_copy(w.bitcast(U32).at[:, i * per_blk + t, :],
                                      wqkv.at[m * HP + i * per_blk + t],
                                      sem_qkv.at[m * HP + i * per_blk + t])
                for m, w in enumerate((wq_hbm, wk_hbm, wv_hbm)) for t in range(per_blk)]

    def wo_copy(n):
        cols = pl.ds(pl.multiple_of(n * 128, 128), 128)
        return pltpu.make_async_copy(wo_hbm.at[:, :, cols], wo.at[n], sem_wo.at[n])

    for cp in (cp_x[:1] + [cp_gw] + cp_w1[:X1_AT] + cp_x[1:2] + cp_w1[X1_AT:] + cp_x[2:]
               + [cp_w2, cp_mem, cp_w3, cp_w4]):
        cp.start()

    def after(dep, x):
        always = (pltpu.bitcast(dep, U32) | U32(1)) != U32(0)
        reps = (x.shape[0] // dep.shape[0], x.shape[1] // dep.shape[1])
        return jnp.where(jnp.tile(always, reps), x, jnp.zeros_like(x))

    def spread(deps, x):
        n = x.shape[0] // len(deps)
        return jnp.concatenate([after(d, x[i * n:(i + 1) * n]) for i, d in enumerate(deps)], axis=0)

    def marks(y):
        pts = [divmod(u * MARK_END // N_MARKS, SUB) for u in range(N_MARKS)]
        return [y[r * (R // SUB):r * (R // SUB) + 8, n * 128:(n + 1) * 128] for n, r in pts]

    lhs = (lhs0, lhs1)
    hbuf[:, 0:HALO, :] = jnp.zeros((n_tiles, HALO, 128), F32)
    hbuf[:, HALO + S:, :] = jnp.zeros((n_tiles, HALO, 128), F32)

    def store_h(rs, h):
        for n in range(n_tiles):
            hbuf[n, rs, :] = h[:, n * 128:(n + 1) * 128]

    def rows(i, offset=0, extra=0):
        return pl.ds(pl.multiple_of(i * R + offset, 8), R + extra)

    def prepare1(i, slot, deps):
        x = ax[rows(i), :].astype(F32)
        if deps is not None:
            x = spread(deps, x)
        gw = gw_ref[...].reshape(1, D).astype(F32)
        g = jax.nn.sigmoid(jnp.sum(x * gw, axis=-1, keepdims=True))
        gate[rows(i), :] = jnp.broadcast_to(g, (R, 128))
        lhs[slot][...] = _layernorm(x).astype(BF16)

    def stage1(i, slot):
        pre = _dot(lhs[slot][...], w1[...])
        store_h(rows(i, HALO), _gelu(pre))
        prepare1(jnp.minimum(i + 1, n_x - 1), 1 - slot, marks(pre))

    def pair1(j, carry):
        for k in range(2, n_x // 2):
            pl.when(j + 1 == k)(cp_x[k + 1].wait)
        stage1(2 * j, 0)
        stage1(2 * j + 1, 1)
        return carry

    cp_x[0].wait()
    cp_gw.wait()
    prepare1(0, 0, None)
    for i, (cp, rs) in enumerate(zip(cp_w1, w1_rows)):
        if i == X1_AT:
            cp_x[1].wait()
            prepare1(1, 1, None)
        cp.wait()
        pre = _dot(lhs0[:, rs], w1[rs, :])
        if i > 0:
            pre = bres[0:R, :] + pre
        if i < len(cp_w1) - 1:
            bres[0:R, :] = pre
    store_h(rows(0, HALO), _gelu(pre))
    cp_x[2].wait()
    stage1(1, 1)
    lax.fori_loop(1, n_x // 2, pair1, 0)

    c = D // 4

    def prepare2(i, slot, deps):
        for n in range(n_tiles):
            shift = (-1, 1, -2, 2)[n * 128 // c]
            part = hbuf[n, pl.ds(i * R + HALO + shift, R), :]
            if deps is not None:
                part = spread(deps, part)
            lhs[slot][:, n * 128:(n + 1) * 128] = part.astype(BF16)

    def stage2(i, slot):
        hs = _dot(lhs[slot][...], w2[...])
        x1 = ax[rows(i), :].astype(F32) + hs
        bres[rows(i), :] = x1
        outbuf[rows(i), :] = _layernorm(x1).astype(BF16)
        prepare2(jnp.minimum(i + 1, n_x - 1), 1 - slot, marks(hs))

    def group2(j, carry):
        for t in range(GROUP_2):
            stage2(GROUP_2 * j + t, t % 2)
        return carry

    cp_w2.wait()
    for cp in qkv_copies(0) + qkv_copies(1):
        cp.start()
    prepare2(0, 0, None)
    lax.fori_loop(0, n_x // GROUP_2, group2, 0)

    def repack(j, k, dep):
        w = after(dep, wqkv[j, k * 128:(k + 1) * 128, :])
        even = pltpu.bitcast(w << 16, F32).astype(BF16)
        odd = pltpu.bitcast(w & U32(0xFFFF0000), F32).astype(BF16)
        wqkv[j, k * 128:k * 128 + 64, :] = pltpu.bitcast(even, U32)
        wqkv[j, k * 128 + 64:(k + 1) * 128, :] = pltpu.bitcast(odd, U32)

    def mlp_body(i, carry):
        for cp in qkv_copies(i):
            cp.wait()
        pre = _dot(outbuf[rows(i), :], w3[...])
        todo = [(m * HP + i * per_blk + t, k)
                for m in range(3) for t in range(per_blk) for k in range(n_tiles)]
        for u, (j, k) in enumerate(todo):
            n, r = divmod(u * 2 * (F // 128) // len(todo), 2)
            repack(j, k, pre[r * (R // 2):r * (R // 2) + 8, n * 128:(n + 1) * 128])
        y = _dot(_gelu(pre).astype(BF16), w4[...])
        bres[rows(i), :] = (1.0 - jnp.tile(gate[rows(i), :], (1, n_tiles))) * (bres[rows(i), :] + y)
        wo_copy(i).start()

        @pl.when(i + 2 < n_blk)
        def _():
            for cp in qkv_copies(i + 2):
                cp.start()

        return carry

    cp_w3.wait()
    cp_w4.wait()
    lax.fori_loop(0, n_blk, mlp_body, 0)
    for n in range(n_tiles):
        wo_copy(n).wait()

    def head_weight(i, h):
        j = i * HP + h // 2
        off = (h % 2) * 64
        w = jnp.concatenate(
            [wqkv[j, k * 128 + off:k * 128 + off + 64, :] for k in range(n_tiles)], axis=0)
        return pltpu.bitcast(w, BF16)

    row = lax.broadcasted_iota(jnp.int32, (L, L), 0)
    col = lax.broadcasted_iota(jnp.int32, (L, L), 1)
    mask = (row < M) | (row >= col)

    cp_mem.wait()
    hseg[0:M, :] = mem0_ref[0].astype(F32)

    def out_copy(r):
        return pltpu.make_async_copy(outbuf.at[pl.ds(r, seg)], out_hbm.at[0, pl.ds(r, seg)],
                                     sem_out)

    def seg_body(s, carry):
        r = pl.multiple_of(s * seg, seg)
        hseg[M:L, :] = ax[pl.ds(r, seg), :].astype(F32)
        qkv = {}
        probs = {}

        def project(h):
            hh = hseg[...]
            ws = [head_weight(i, h) for i in range(3)]
            if h == 0:
                k = D // 2
                part = [_dot(hh[:, :k], w[:k]) for w in ws]
                oacc[:, 0:3 * E] = jnp.concatenate(part, axis=1)
                qkv[h] = [oacc[:, i * E:(i + 1) * E] + _dot(hh[:, k:], w[k:]) for i, w in enumerate(ws)]
            else:
                qkv[h] = [_dot(hh, w) for w in ws]

        def scores(h):
            q, k, _ = qkv[h]
            sc = jnp.where(mask, _dot_nt(q, k) * scale, -1000000000.0)
            e = jnp.exp(sc - jnp.max(sc, axis=-1, keepdims=True))
            probs[h] = e / jnp.sum(e, axis=-1, keepdims=True)

        def values(h):
            obuf[:, h * E:(h + 1) * E] = _dot(probs.pop(h), qkv.pop(h)[2])

        def out_part(h0, h1, n):
            w = wo[n, h0:h1].reshape((h1 - h0) * E, 128)
            return _dot(obuf[:, h0 * E:h1 * E], w)

        for h in range(H):
            project(h)
            if h >= 1:
                scores(h - 1)
            if h >= 3:
                values(h - 3)
        half = H // 2
        tail = {0: [(scores, H - 1), (values, H - 3)], 2: [(values, H - 2)], 3: [(values, H - 1)]}
        for n in range(n_tiles):
            oacc[:, n * 128:(n + 1) * 128] = out_part(0, half, n)
            for fn, h in tail.get(n, ()):
                fn(h)
        g = gate[pl.ds(r, seg), :]
        for n in range(n_tiles):
            cols = slice(n * 128, (n + 1) * 128)
            o = oacc[:, cols] + out_part(half, H, n)
            hseg[0:M, cols] = o[0:M]
            outbuf[pl.ds(r, seg), cols] = (g * o[M:L] + bres[pl.ds(r, seg), cols]).astype(BF16)
        out_copy(r).start()
        return carry

    lax.fori_loop(0, n_seg, seg_body, 0, unroll=SEG_UNROLL)
    pltpu.make_async_copy(outbuf, out_hbm.at[0], sem_out).wait()


@functools.partial(jax.jit, static_argnames=("A_seg_len",))
def pallas_gated_mix__memory_aug_recurrent_mem_tr__mixer_s_mlp__prompt_kernel(
    A_x: jax.Array,
    A_mem0: jax.Array,
    A_Wq: jax.Array,
    A_Wk: jax.Array,
    A_Wv: jax.Array,
    A_Wo: jax.Array,
    A_seg_len: int,
    B_x: jax.Array,
    B_w1: jax.Array,
    B_w2: jax.Array,
    B_w3: jax.Array,
    B_w4: jax.Array,
    gate_w: jax.Array,
):
    _, S, D = A_x.shape
    _, H, E = A_Wq.shape
    M = A_mem0.shape[1]
    F = B_w3.shape[1]
    seg = int(A_seg_len)
    hbm = pl.BlockSpec(memory_space=pl.ANY)
    return pl.pallas_call(
        functools.partial(_kernel, seg=seg),
        out_shape=jax.ShapeDtypeStruct(A_x.shape, A_x.dtype),
        in_specs=[hbm] * 11,
        out_specs=hbm,
        scratch_shapes=[
            pltpu.VMEM((3 * H // 2, D, E), U32),
            pltpu.VMEM((D // 128, H, E, 128), BF16),
            pltpu.VMEM((D, D), BF16),
            pltpu.VMEM((D, D), BF16),
            pltpu.VMEM((D, F), BF16),
            pltpu.VMEM((F, D), BF16),
            pltpu.VMEM((S, D), BF16),
            pltpu.VMEM((D // 128, S + 2 * HALO, 128), F32),
            pltpu.VMEM((S, D), F32),
            pltpu.VMEM((S, 128), F32),
            pltpu.VMEM((M + seg, D), F32),
            pltpu.VMEM((M + seg, H * E), F32),
            pltpu.VMEM((M + seg, D), F32),
            pltpu.VMEM((S, D), BF16),
            pltpu.VMEM((ROWS_X, D), BF16),
            pltpu.VMEM((ROWS_X, D), BF16),
            pltpu.VMEM(A_mem0.shape, BF16),
            pltpu.VMEM(gate_w.shape, BF16),
            pltpu.SemaphoreType.DMA((S // ROWS_X + len(W1_SPLIT) + 4,)),
            pltpu.SemaphoreType.DMA((3 * H // 2,)),
            pltpu.SemaphoreType.DMA((D // 128,)),
            pltpu.SemaphoreType.DMA(()),
        ],
        compiler_params=pltpu.CompilerParams(vmem_limit_bytes=120 * 1024 * 1024, disable_bounds_checks=True),
    )(A_x, A_mem0, A_Wq, A_Wk, A_Wv, A_Wo, B_w1, B_w2, B_w3, B_w4, gate_w)
```

```python
import functools

import jax
import jax.numpy as jnp
from jax import lax
import jax.experimental.pallas as pl
import jax.experimental.pallas.tpu as pltpu

F32 = jnp.float32
BF16 = jnp.bfloat16
U32 = jnp.uint32

LANES = 128
ROWS = 256
W1_SPLIT = (0, 256, 512, 1024)
GROUP_2 = 4
SEG_UNROLL = 2
HALO = 8
SHIFTS = (-1, 1, -2, 2)


def _dot(a, b):
    return lax.dot_general(a, b, (((1,), (0,)), ((), ())), preferred_element_type=F32)


def _dot_nt(a, b):
    return lax.dot_general(a, b, (((1,), (1,)), ((), ())), preferred_element_type=F32)


def _layernorm(x, eps=1e-05):
    m = jnp.mean(x, axis=-1, keepdims=True)
    c = x - m
    v = jnp.mean(c * c, axis=-1, keepdims=True)
    return c * lax.rsqrt(v + eps)


def _gelu(x):
    return jax.nn.gelu(x, approximate=True)


def _after(dep, x):
    always = (pltpu.bitcast(dep, U32) | U32(1)) != U32(0)
    reps = (x.shape[0] // dep.shape[0], x.shape[1] // dep.shape[1])
    return jnp.where(jnp.tile(always, reps), x, jnp.zeros_like(x))


def _mark(y, step, per_tile):
    n, r = divmod(step, per_tile)
    r *= y.shape[0] // per_tile
    return y[r:r + 8, n * LANES:(n + 1) * LANES]


def _during(y, x):
    pieces, per_tile = x.shape[0] // 8, 4
    steps = (y.shape[1] // LANES - 1) * per_tile
    return jnp.concatenate(
        [_after(_mark(y, i * steps // pieces, per_tile), x[8 * i:8 * i + 8])
         for i in range(pieces)], axis=0)


def _kernel(x_hbm, mem0_hbm, wq_hbm, wk_hbm, wv_hbm, wo_hbm, w1_hbm, w2_hbm, w3_hbm, w4_hbm,
            gw_hbm, out_hbm,
            wqkv, wo, w1, w2, w3, w4, xs, hbuf, lhs0, lhs1, bres,
            gate, outbuf, hseg, obuf, oacc, mem0, gw, sem_in, sem_qkv, sem_wo, sem_out, *, seg):
    S, D = xs.shape
    _, H, E = wq_hbm.shape
    M = mem0.shape[1]
    L = M + seg
    F = w3.shape[1]
    R = ROWS
    n_blk = S // R
    n_tiles = D // LANES
    pairs = H // 2
    pairs_per_blk = pairs // n_blk
    assert E == LANES and n_blk == n_tiles and pairs % n_blk == 0 and H >= 8
    assert S % (GROUP_2 * R) == 0 and GROUP_2 % 2 == 0 and W1_SPLIT[-1] == D
    assert M % 8 == 0 and seg % 16 == 0 and S % (SEG_UNROLL * seg) == 0

    def copy(src, dst, i):
        return pltpu.make_async_copy(src, dst, sem_in.at[i])

    x_rows = [pl.ds(i * R, R) for i in range(3)]
    x_rows += [pl.ds(i * R, min(2 * R, S - i * R)) for i in range(3, n_blk, 2)]
    w1_rows = [slice(r0, r1) for r0, r1 in zip(W1_SPLIT, W1_SPLIT[1:])]
    cp_x = [copy(x_hbm.at[0, rs], xs.at[rs], i) for i, rs in enumerate(x_rows)]
    cp_w1 = [copy(w1_hbm.at[rs], w1.at[rs], n_blk + i) for i, rs in enumerate(w1_rows)]
    cp_w2, cp_w3, cp_w4, cp_gw, cp_mem = [
        copy(src, dst, n_blk + len(w1_rows) + i) for i, (src, dst) in enumerate(
            ((w2_hbm, w2), (w3_hbm, w3), (w4_hbm, w4), (gw_hbm, gw), (mem0_hbm, mem0)))]

    def slabs(i):
        return [(w, (m, i * pairs_per_blk + t))
                for m, w in enumerate((wq_hbm, wk_hbm, wv_hbm)) for t in range(pairs_per_blk)]

    def qkv_copies(i):
        return [pltpu.make_async_copy(w.bitcast(U32).at[:, p, :], wqkv.at[m * pairs + p],
                                      sem_qkv.at[m * pairs + p])
                for w, (m, p) in slabs(i)]

    def wo_copy(n):
        cols = pl.ds(pl.multiple_of(n * LANES, LANES), LANES)
        return pltpu.make_async_copy(wo_hbm.at[:, :, cols], wo.at[n], sem_wo.at[n])

    for cp in ([cp_x[0], cp_gw, cp_w1[0], cp_x[1]] + cp_w1[1:] + cp_x[2:]
               + [cp_w2, cp_mem, cp_w3, cp_w4]):
        cp.start()

    def rows(i, offset=0):
        return pl.ds(pl.multiple_of(i * R + offset, 8), R)

    lhs = (lhs0, lhs1)
    hbuf[:, 0:HALO, :] = jnp.zeros((n_tiles, HALO, LANES), F32)
    hbuf[:, HALO + S:, :] = jnp.zeros((n_tiles, HALO, LANES), F32)

    def prepare1(i, slot, y=None):
        x = xs[rows(i), :].astype(F32)
        if y is not None:
            x = _during(y, x)
        logit = jnp.sum(x * gw[...].reshape(1, D).astype(F32), axis=-1, keepdims=True)
        gate[rows(i), :] = jnp.broadcast_to(jax.nn.sigmoid(logit), (R, LANES))
        lhs[slot][...] = _layernorm(x).astype(BF16)

    def store_h(i, pre):
        h = _gelu(pre)
        for n in range(n_tiles):
            hbuf[n, rows(i, HALO), :] = h[:, n * LANES:(n + 1) * LANES]

    k0, k1, k2 = w1_rows
    cp_x[0].wait()
    cp_gw.wait()
    prepare1(0, 0)
    cp_w1[0].wait()
    bres[0:R, :] = _dot(lhs0[:, k0], w1[k0, :])
    cp_x[1].wait()
    prepare1(1, 1)
    cp_w1[1].wait()
    bres[0:R, :] += _dot(lhs0[:, k1], w1[k1, :])
    bres[R:2 * R, :] = _dot(lhs1[:, :k1.stop], w1[:k1.stop, :])
    cp_w1[2].wait()
    cp_x[2].wait()
    for i in range(2):
        pre = bres[i * R:(i + 1) * R, :] + _dot(lhs[i][:, k2], w1[k2, :])
        store_h(i, pre)
    prepare1(2, 0, pre)

    def step1(j, carry):
        for k in range(1, n_blk // 2):
            pl.when(j == k)(cp_x[k + 2].wait)
        for slot in range(2):
            i = 2 * j + slot
            pre = _dot(lhs[slot][...], w1[...])
            store_h(i, pre)
            prepare1(jnp.minimum(i + 1, n_blk - 1), 1 - slot, pre)
        return carry

    lax.fori_loop(1, n_blk // 2, step1, 0)

    def prepare2(i, slot, y=None):
        for n in range(n_tiles):
            shift = SHIFTS[n * len(SHIFTS) // n_tiles]
            part = hbuf[n, pl.ds(i * R + HALO + shift, R), :]
            if y is not None:
                part = _during(y, part)
            lhs[slot][:, n * LANES:(n + 1) * LANES] = part.astype(BF16)

    def step2(j, carry):
        x1 = None
        for t in range(GROUP_2):
            i = GROUP_2 * j + t
            hs = _dot(lhs[t % 2][...], w2[...])
            if x1 is not None:
                outbuf[rows(i - 1), :] = _layernorm(_during(hs, x1)).astype(BF16)
            x1 = xs[rows(i), :].astype(F32) + hs
            bres[rows(i), :] = x1
            prepare2(jnp.minimum(i + 1, n_blk - 1), 1 - t % 2, hs)
        outbuf[rows(i), :] = _layernorm(x1).astype(BF16)
        return carry

    cp_w2.wait()
    for cp in qkv_copies(0) + qkv_copies(1):
        cp.start()
    prepare2(0, 0)
    lax.fori_loop(0, n_blk // GROUP_2, step2, 0)

    def repack(j, k, dep):
        r = k * LANES
        w = _after(dep, wqkv[j, r:r + LANES, :])
        even = pltpu.bitcast(w << 16, F32).astype(BF16)
        odd = pltpu.bitcast(w & U32(0xFFFF0000), F32).astype(BF16)
        wqkv[j, r:r + LANES // 2, :] = pltpu.bitcast(even, U32)
        wqkv[j, r + LANES // 2:r + LANES, :] = pltpu.bitcast(odd, U32)

    def step3(i, carry):
        for cp in qkv_copies(i):
            cp.wait()
        pre = _dot(outbuf[rows(i), :], w3[...])
        todo = [(m * pairs + p, k) for _, (m, p) in slabs(i) for k in range(n_tiles)]
        for u, (j, k) in enumerate(todo):
            repack(j, k, _mark(pre, u * 2 * (F // LANES) // len(todo), 2))
        y = _dot(_gelu(pre), w4[...])
        g = jnp.tile(gate[rows(i), :], (1, n_tiles))
        bres[rows(i), :] = (1.0 - g) * (bres[rows(i), :] + y)
        wo_copy(i).start()

        @pl.when(i + 2 < n_blk)
        def _():
            for cp in qkv_copies(i + 2):
                cp.start()

        return carry

    cp_w3.wait()
    cp_w4.wait()
    lax.fori_loop(0, n_blk, step3, 0)
    for n in range(n_tiles):
        wo_copy(n).wait()

    def head_weight(m, h):
        j, off = m * pairs + h // 2, (h % 2) * (LANES // 2)
        w = jnp.concatenate(
            [wqkv[j, k * LANES + off:k * LANES + off + LANES // 2, :] for k in range(n_tiles)],
            axis=0)
        return pltpu.bitcast(w, BF16)

    row = lax.broadcasted_iota(jnp.int32, (L, L), 0)
    col = lax.broadcasted_iota(jnp.int32, (L, L), 1)
    mask = (row < M) | (row >= col)

    cp_mem.wait()
    hseg[0:M, :] = mem0[0].astype(F32)

    def step4(s, carry):
        tokens = pl.ds(pl.multiple_of(s * seg, seg), seg)
        hseg[M:L, :] = xs[tokens, :].astype(F32)
        qkv = {}
        probs = {}

        def project(h):
            hh = hseg[...]
            ws = [head_weight(m, h) for m in range(3)]
            if h == 0:
                k = D // 2
                oacc[:, 0:3 * E] = jnp.concatenate([_dot(hh[:, :k], w[:k]) for w in ws], axis=1)
                qkv[h] = [oacc[:, m * E:(m + 1) * E] + _dot(hh[:, k:], w[k:])
                          for m, w in enumerate(ws)]
            else:
                qkv[h] = [_dot(hh, w) for w in ws]

        def scores(h):
            q, k, _ = qkv[h]
            sc = jnp.where(mask, _dot_nt(q, k) * E ** (-0.5), -1000000000.0)
            e = jnp.exp(sc - jnp.max(sc, axis=-1, keepdims=True))
            probs[h] = e / jnp.sum(e, axis=-1, keepdims=True)

        def values(h):
            obuf[:, h * E:(h + 1) * E] = _dot(probs.pop(h), qkv.pop(h)[2])

        def out_part(h0, h1, n):
            return _dot(obuf[:, h0 * E:h1 * E], wo[n, h0:h1].reshape((h1 - h0) * E, LANES))

        for h in range(H):
            project(h)
            if h >= 1:
                scores(h - 1)
            if h >= 3:
                values(h - 3)
        late = {0: [(scores, H - 1), (values, H - 3)], 2: [(values, H - 2)], 3: [(values, H - 1)]}
        for n in range(n_tiles):
            oacc[:, n * LANES:(n + 1) * LANES] = out_part(0, H // 2, n)
            for fn, h in late.get(n, ()):
                fn(h)
        g = gate[tokens, :]
        for n in range(n_tiles):
            cols = slice(n * LANES, (n + 1) * LANES)
            o = oacc[:, cols] + out_part(H // 2, H, n)
            hseg[0:M, cols] = o[0:M]
            outbuf[tokens, cols] = (g * o[M:L] + bres[tokens, cols]).astype(outbuf.dtype)
        pltpu.make_async_copy(outbuf.at[tokens], out_hbm.at[0, tokens], sem_out).start()
        return carry

    lax.fori_loop(0, S // seg, step4, 0, unroll=SEG_UNROLL)
    pltpu.make_async_copy(outbuf, out_hbm.at[0], sem_out).wait()


@functools.partial(jax.jit, static_argnames=("A_seg_len",))
def pallas_gated_mix__memory_aug_recurrent_mem_tr__mixer_s_mlp__prompt_kernel(
    A_x: jax.Array,
    A_mem0: jax.Array,
    A_Wq: jax.Array,
    A_Wk: jax.Array,
    A_Wv: jax.Array,
    A_Wo: jax.Array,
    A_seg_len: int,
    B_x: jax.Array,
    B_w1: jax.Array,
    B_w2: jax.Array,
    B_w3: jax.Array,
    B_w4: jax.Array,
    gate_w: jax.Array,
):
    del B_x
    batch, S, D = A_x.shape
    _, H, E = A_Wq.shape
    F = B_w3.shape[1]
    seg = int(A_seg_len)
    L = A_mem0.shape[1] + seg
    assert batch == 1 and A_x.dtype == BF16
    hbm = pl.BlockSpec(memory_space=pl.ANY)
    return pl.pallas_call(
        functools.partial(_kernel, seg=seg),
        out_shape=jax.ShapeDtypeStruct(A_x.shape, A_x.dtype),
        in_specs=[hbm] * 11,
        out_specs=hbm,
        scratch_shapes=[
            pltpu.VMEM((3 * H // 2, D, E), U32),
            pltpu.VMEM((D // LANES, H, E, LANES), BF16),
            pltpu.VMEM((D, D), BF16),
            pltpu.VMEM((D, D), BF16),
            pltpu.VMEM((D, F), BF16),
            pltpu.VMEM((F, D), BF16),
            pltpu.VMEM((S, D), BF16),
            pltpu.VMEM((D // LANES, S + 2 * HALO, LANES), F32),
            pltpu.VMEM((ROWS, D), BF16),
            pltpu.VMEM((ROWS, D), BF16),
            pltpu.VMEM((S, D), F32),
            pltpu.VMEM((S, LANES), F32),
            pltpu.VMEM((S, D), BF16),
            pltpu.VMEM((L, D), F32),
            pltpu.VMEM((L, H * E), F32),
            pltpu.VMEM((L, D), F32),
            pltpu.VMEM(A_mem0.shape, BF16),
            pltpu.VMEM(gate_w.shape, BF16),
            pltpu.SemaphoreType.DMA((S // ROWS + len(W1_SPLIT) + 4,)),
            pltpu.SemaphoreType.DMA((3 * H // 2,)),
            pltpu.SemaphoreType.DMA((D // LANES,)),
            pltpu.SemaphoreType.DMA(()),
        ],
        compiler_params=pltpu.CompilerParams(
            vmem_limit_bytes=120 * 1024 * 1024, disable_bounds_checks=True),
    )(A_x, A_mem0, A_Wq, A_Wk, A_Wv, A_Wo, B_w1, B_w2, B_w3, B_w4, gate_w)
```

```python
import functools

import jax
import jax.numpy as jnp
from jax import lax
import jax.experimental.pallas as pl
import jax.experimental.pallas.tpu as pltpu

F32 = jnp.float32
BF16 = jnp.bfloat16
U32 = jnp.uint32

LANES = 128
ROWS = 256
W1_SPLIT = (0, 256, 512, 1024)
GROUP_2 = 4
LAST_PARTS = 4
SEG_UNROLL = 4
HALO = 8
SHIFTS = (-1, 1, -2, 2)


def _dot(a, b):
    return lax.dot_general(a, b, (((1,), (0,)), ((), ())), preferred_element_type=F32)


def _dot_nt(a, b):
    return lax.dot_general(a, b, (((1,), (1,)), ((), ())), preferred_element_type=F32)


def _layernorm(x, eps=1e-05):
    m = jnp.mean(x, axis=-1, keepdims=True)
    c = x - m
    v = jnp.mean(c * c, axis=-1, keepdims=True)
    return c * lax.rsqrt(v + eps)


def _gelu(x):
    return jax.nn.gelu(x, approximate=True)


def _after(dep, x):
    always = (pltpu.bitcast(dep, U32) | U32(1)) != U32(0)
    reps = (x.shape[0] // dep.shape[0], x.shape[1] // dep.shape[1])
    return jnp.where(jnp.tile(always, reps), x, jnp.zeros_like(x))


def _mark(y, step, per_tile):
    n, r = divmod(step, per_tile)
    r *= y.shape[0] // per_tile
    return y[r:r + 8, n * LANES:(n + 1) * LANES]


def _during(y, x):
    pieces, per_tile = x.shape[0] // 8, 4
    steps = (y.shape[1] // LANES - 1) * per_tile
    return jnp.concatenate(
        [_after(_mark(y, i * steps // pieces, per_tile), x[8 * i:8 * i + 8])
         for i in range(pieces)], axis=0)


def _kernel(x_hbm, mem0_hbm, wq_hbm, wk_hbm, wv_hbm, wo_hbm, w1_hbm, w2_hbm, w3_hbm, w4_hbm,
            gw_hbm, out_hbm,
            wqkv, wo, w1, w2, w3, w4, xs, hbuf, lhs0, lhs1, bres,
            gate, outbuf, hseg, obuf, oacc, mem0, gw, sem_in, sem_qkv, sem_wo, sem_out, *, seg):
    S, D = xs.shape
    _, H, E = wq_hbm.shape
    M = mem0.shape[1]
    L = M + seg
    F = w3.shape[1]
    R = ROWS
    n_blk = S // R
    n_tiles = D // LANES
    pairs = H // 2
    pairs_per_blk = pairs // n_blk
    assert E == LANES and n_blk == n_tiles and pairs % n_blk == 0 and H >= 8
    assert S % (GROUP_2 * R) == 0 and GROUP_2 % 2 == 0 and W1_SPLIT[-1] == D
    assert F % (LAST_PARTS * LANES) == 0 and n_tiles % LAST_PARTS == 0
    assert M % 8 == 0 and seg % 16 == 0 and S % (SEG_UNROLL * seg) == 0

    def copy(src, dst, i):
        return pltpu.make_async_copy(src, dst, sem_in.at[i])

    x_rows = [pl.ds(i * R, R) for i in range(3)]
    x_rows += [pl.ds(i * R, min(2 * R, S - i * R)) for i in range(3, n_blk, 2)]
    w1_rows = [slice(r0, r1) for r0, r1 in zip(W1_SPLIT, W1_SPLIT[1:])]
    cp_x = [copy(x_hbm.at[0, rs], xs.at[rs], i) for i, rs in enumerate(x_rows)]
    cp_w1 = [copy(w1_hbm.at[rs], w1.at[rs], n_blk + i) for i, rs in enumerate(w1_rows)]
    cp_w2, cp_w3, cp_w4, cp_gw, cp_mem = [
        copy(src, dst, n_blk + len(w1_rows) + i) for i, (src, dst) in enumerate(
            ((w2_hbm, w2), (w3_hbm, w3), (w4_hbm, w4), (gw_hbm, gw), (mem0_hbm, mem0)))]

    def slabs(i):
        return [(w, (m, i * pairs_per_blk + t))
                for m, w in enumerate((wq_hbm, wk_hbm, wv_hbm)) for t in range(pairs_per_blk)]

    def qkv_copies(i):
        return [pltpu.make_async_copy(w.bitcast(U32).at[:, p, :], wqkv.at[m * pairs + p],
                                      sem_qkv.at[m * pairs + p])
                for w, (m, p) in slabs(i)]

    def wo_copy(n):
        cols = pl.ds(pl.multiple_of(n * LANES, LANES), LANES)
        return pltpu.make_async_copy(wo_hbm.at[:, :, cols], wo.at[n], sem_wo.at[n])

    for cp in ([cp_x[0], cp_gw, cp_w1[0], cp_x[1]] + cp_w1[1:] + cp_x[2:]
               + [cp_w2, cp_mem, cp_w3, cp_w4]):
        cp.start()

    def rows(i, offset=0):
        return pl.ds(pl.multiple_of(i * R + offset, 8), R)

    lhs = (lhs0, lhs1)
    hbuf[:, 0:HALO, :] = jnp.zeros((n_tiles, HALO, LANES), F32)
    hbuf[:, HALO + S:, :] = jnp.zeros((n_tiles, HALO, LANES), F32)

    def prepare1(i, slot, y=None):
        x = xs[rows(i), :].astype(F32)
        if y is not None:
            x = _during(y, x)
        logit = jnp.sum(x * gw[...].reshape(1, D).astype(F32), axis=-1, keepdims=True)
        gate[rows(i), :] = jnp.broadcast_to(jax.nn.sigmoid(logit), (R, LANES))
        lhs[slot][...] = _layernorm(x).astype(BF16)

    def store_h(i, pre):
        h = _gelu(pre)
        for n in range(n_tiles):
            hbuf[n, rows(i, HALO), :] = h[:, n * LANES:(n + 1) * LANES]

    k0, k1, k2 = w1_rows
    cp_x[0].wait()
    cp_gw.wait()
    prepare1(0, 0)
    cp_w1[0].wait()
    bres[0:R, :] = _dot(lhs0[:, k0], w1[k0, :])
    cp_x[1].wait()
    prepare1(1, 1)
    cp_w1[1].wait()
    bres[0:R, :] += _dot(lhs0[:, k1], w1[k1, :])
    bres[R:2 * R, :] = _dot(lhs1[:, :k1.stop], w1[:k1.stop, :])
    cp_w1[2].wait()
    cp_x[2].wait()
    for i in range(2):
        pre = bres[i * R:(i + 1) * R, :] + _dot(lhs[i][:, k2], w1[k2, :])
        store_h(i, pre)
    prepare1(2, 0, pre)

    def step1(j, carry):
        for k in range(1, n_blk // 2):
            pl.when(j == k)(cp_x[k + 2].wait)
        for slot in range(2):
            i = 2 * j + slot
            pre = _dot(lhs[slot][...], w1[...])
            store_h(i, pre)
            prepare1(jnp.minimum(i + 1, n_blk - 1), 1 - slot, pre)
        return carry

    lax.fori_loop(1, n_blk // 2, step1, 0)

    def prepare2(i, slot, y=None):
        for n in range(n_tiles):
            shift = SHIFTS[n * len(SHIFTS) // n_tiles]
            part = hbuf[n, pl.ds(i * R + HALO + shift, R), :]
            if y is not None:
                part = _during(y, part)
            lhs[slot][:, n * LANES:(n + 1) * LANES] = part.astype(BF16)

    def step2(j, carry):
        x1 = None
        for t in range(GROUP_2):
            i = GROUP_2 * j + t
            hs = _dot(lhs[t % 2][...], w2[...])
            if x1 is not None:
                outbuf[rows(i - 1), :] = _layernorm(_during(hs, x1)).astype(BF16)
            x1 = xs[rows(i), :].astype(F32) + hs
            bres[rows(i), :] = x1
            prepare2(jnp.minimum(i + 1, n_blk - 1), 1 - t % 2, hs)
        outbuf[rows(i), :] = _layernorm(x1).astype(BF16)
        return carry

    cp_w2.wait()
    for cp in qkv_copies(0) + qkv_copies(1):
        cp.start()
    prepare2(0, 0)
    lax.fori_loop(0, n_blk // GROUP_2, step2, 0)

    def repack(j, k, dep):
        half = LANES // 2
        r = pl.multiple_of(k * LANES, LANES)
        w = _after(dep, wqkv[j, pl.ds(r, LANES), :])
        even = pltpu.bitcast(w << 16, F32).astype(BF16)
        odd = pltpu.bitcast(w & U32(0xFFFF0000), F32).astype(BF16)
        wqkv[j, pl.ds(r, half), :] = pltpu.bitcast(even, U32)
        wqkv[j, pl.ds(pl.multiple_of(r + half, half), half), :] = pltpu.bitcast(odd, U32)

    def mlp(i, q, parts):
        width = F // parts
        fs = pl.ds(pl.multiple_of(q * width, LANES), width)
        pre = _dot(outbuf[rows(i), :], w3[:, fs])
        todo = [(m * pairs + p, q * (n_tiles // parts) + t)
                for _, (m, p) in slabs(i) for t in range(n_tiles // parts)]
        for u, (j, k) in enumerate(todo):
            repack(j, k, _mark(pre, u * 2 * (width // LANES) // len(todo), 2))
        bres[rows(i), :] += _dot(_gelu(pre), w4[fs, :])

    def step3(i, carry):
        for cp in qkv_copies(i):
            cp.wait()
        mlp(i, 0, 1)
        wo_copy(i).start()

        @pl.when(i + 2 < n_blk)
        def _():
            for cp in qkv_copies(i + 2):
                cp.start()

        return carry

    cp_w3.wait()
    cp_w4.wait()
    lax.fori_loop(0, n_blk - 1, step3, 0)
    wo_copy(n_blk - 1).start()
    for cp in qkv_copies(n_blk - 1):
        cp.wait()
    lax.fori_loop(0, LAST_PARTS, lambda q, _: mlp(n_blk - 1, q, LAST_PARTS), None)
    for n in range(n_tiles):
        wo_copy(n).wait()

    def head_weight(m, h):
        j, off = m * pairs + h // 2, (h % 2) * (LANES // 2)
        w = jnp.concatenate(
            [wqkv[j, k * LANES + off:k * LANES + off + LANES // 2, :] for k in range(n_tiles)],
            axis=0)
        return pltpu.bitcast(w, BF16)

    row = lax.broadcasted_iota(jnp.int32, (L, L), 0)
    col = lax.broadcasted_iota(jnp.int32, (L, L), 1)
    mask = (row < M) | (row >= col)

    cp_mem.wait()
    hseg[0:M, :] = mem0[0].astype(F32)

    def step4(s, carry):
        tokens = pl.ds(pl.multiple_of(s * seg, seg), seg)
        hseg[M:L, :] = xs[tokens, :].astype(F32)
        qkv = {}
        probs = {}

        def project(h):
            hh = hseg[...]
            ws = [head_weight(m, h) for m in range(3)]
            if h == 0:
                k = D // 2
                oacc[:, 0:3 * E] = jnp.concatenate([_dot(hh[:, :k], w[:k]) for w in ws], axis=1)
                qkv[h] = [oacc[:, m * E:(m + 1) * E] + _dot(hh[:, k:], w[k:])
                          for m, w in enumerate(ws)]
            else:
                qkv[h] = [_dot(hh, w) for w in ws]

        def scores(h):
            q, k, _ = qkv[h]
            sc = jnp.where(mask, _dot_nt(q, k) * E ** (-0.5), -1000000000.0)
            e = jnp.exp(sc - jnp.max(sc, axis=-1, keepdims=True))
            probs[h] = e / jnp.sum(e, axis=-1, keepdims=True)

        def values(h):
            obuf[:, h * E:(h + 1) * E] = _dot(probs.pop(h), qkv.pop(h)[2])

        def out_part(h0, h1, n):
            return _dot(obuf[:, h0 * E:h1 * E], wo[n, h0:h1].reshape((h1 - h0) * E, LANES))

        for h in range(H):
            project(h)
            if h >= 1:
                scores(h - 1)
            if h >= 3:
                values(h - 3)
        late = {0: [(scores, H - 1), (values, H - 3)], 2: [(values, H - 2)], 3: [(values, H - 1)]}
        for n in range(n_tiles):
            oacc[:, n * LANES:(n + 1) * LANES] = out_part(0, H // 2, n)
            for fn, h in late.get(n, ()):
                fn(h)
        g = gate[tokens, :]
        for n in range(n_tiles):
            cols = slice(n * LANES, (n + 1) * LANES)
            o = oacc[:, cols] + out_part(H // 2, H, n)
            hseg[0:M, cols] = o[0:M]
            mixed = g * o[M:L] + (1.0 - g) * bres[tokens, cols]
            outbuf[tokens, cols] = mixed.astype(outbuf.dtype)
        pltpu.make_async_copy(outbuf.at[tokens], out_hbm.at[0, tokens], sem_out).start()
        return carry

    lax.fori_loop(0, S // seg, step4, 0, unroll=SEG_UNROLL)
    pltpu.make_async_copy(outbuf, out_hbm.at[0], sem_out).wait()


@functools.partial(jax.jit, static_argnames=("A_seg_len",))
def pallas_gated_mix__memory_aug_recurrent_mem_tr__mixer_s_mlp__prompt_kernel(
    A_x: jax.Array,
    A_mem0: jax.Array,
    A_Wq: jax.Array,
    A_Wk: jax.Array,
    A_Wv: jax.Array,
    A_Wo: jax.Array,
    A_seg_len: int,
    B_x: jax.Array,
    B_w1: jax.Array,
    B_w2: jax.Array,
    B_w3: jax.Array,
    B_w4: jax.Array,
    gate_w: jax.Array,
):
    del B_x
    batch, S, D = A_x.shape
    _, H, E = A_Wq.shape
    F = B_w3.shape[1]
    seg = int(A_seg_len)
    L = A_mem0.shape[1] + seg
    assert batch == 1 and A_x.dtype == BF16
    hbm = pl.BlockSpec(memory_space=pl.ANY)
    return pl.pallas_call(
        functools.partial(_kernel, seg=seg),
        out_shape=jax.ShapeDtypeStruct(A_x.shape, A_x.dtype),
        in_specs=[hbm] * 11,
        out_specs=hbm,
        scratch_shapes=[
            pltpu.VMEM((3 * H // 2, D, E), U32),
            pltpu.VMEM((D // LANES, H, E, LANES), BF16),
            pltpu.VMEM((D, D), BF16),
            pltpu.VMEM((D, D), BF16),
            pltpu.VMEM((D, F), BF16),
            pltpu.VMEM((F, D), BF16),
            pltpu.VMEM((S, D), BF16),
            pltpu.VMEM((D // LANES, S + 2 * HALO, LANES), F32),
            pltpu.VMEM((ROWS, D), BF16),
            pltpu.VMEM((ROWS, D), BF16),
            pltpu.VMEM((S, D), F32),
            pltpu.VMEM((S, LANES), F32),
            pltpu.VMEM((S, D), BF16),
            pltpu.VMEM((L, D), F32),
            pltpu.VMEM((L, H * E), F32),
            pltpu.VMEM((L, D), F32),
            pltpu.VMEM(A_mem0.shape, BF16),
            pltpu.VMEM(gate_w.shape, BF16),
            pltpu.SemaphoreType.DMA((S // ROWS + len(W1_SPLIT) + 4,)),
            pltpu.SemaphoreType.DMA((3 * H // 2,)),
            pltpu.SemaphoreType.DMA((D // LANES,)),
            pltpu.SemaphoreType.DMA(()),
        ],
        compiler_params=pltpu.CompilerParams(
            vmem_limit_bytes=120 * 1024 * 1024, disable_bounds_checks=True),
    )(A_x, A_mem0, A_Wq, A_Wk, A_Wv, A_Wo, B_w1, B_w2, B_w3, B_w4, gate_w)
```

```python
import functools

import jax
import jax.numpy as jnp
from jax import lax
import jax.experimental.pallas as pl
import jax.experimental.pallas.tpu as pltpu

F32 = jnp.float32
BF16 = jnp.bfloat16
U32 = jnp.uint32

LANES = 128
ROWS = 256
W1_SPLIT = (0, 256, 512, 1024)
GROUP_2 = 4
LAST_PARTS = 4
SEG_UNROLL = 4
HALO = 8
SHIFTS = (-1, 1, -2, 2)


def _dot(a, b):
    return lax.dot_general(a, b, (((1,), (0,)), ((), ())), preferred_element_type=F32)


def _dot_nt(a, b):
    return lax.dot_general(a, b, (((1,), (1,)), ((), ())), preferred_element_type=F32)


def _layernorm(x, eps=1e-05):
    m = jnp.mean(x, axis=-1, keepdims=True)
    c = x - m
    v = jnp.mean(c * c, axis=-1, keepdims=True)
    return c * lax.rsqrt(v + eps)


def _gelu(x):
    return jax.nn.gelu(x, approximate=True)


def _after(dep, x):
    always = (pltpu.bitcast(dep, U32) | U32(1)) != U32(0)
    reps = (x.shape[0] // dep.shape[0], x.shape[1] // dep.shape[1])
    return jnp.where(jnp.tile(always, reps), x, jnp.zeros_like(x))


def _mark(y, step, per_tile):
    n, r = divmod(step, per_tile)
    r *= y.shape[0] // per_tile
    return y[r:r + 8, n * LANES:(n + 1) * LANES]


def _during(y, x):
    pieces, per_tile = x.shape[0] // 8, 4
    steps = (y.shape[1] // LANES - 1) * per_tile
    return jnp.concatenate(
        [_after(_mark(y, i * steps // pieces, per_tile), x[8 * i:8 * i + 8])
         for i in range(pieces)], axis=0)


def _kernel(x_hbm, mem0_hbm, wq_hbm, wk_hbm, wv_hbm, wo_hbm, w1_hbm, w2_hbm, w3_hbm, w4_hbm,
            gw_hbm, out_hbm,
            wqkv, wo, w1, w2, w3, w4, xs, hbuf, lhs0, lhs1, bres,
            gate, outbuf, hseg, obuf, oacc, mem0, gw, sem_in, sem_qkv, sem_wo, sem_out, *, seg):
    S, D = xs.shape
    _, H, E = wq_hbm.shape
    M = mem0.shape[1]
    L = M + seg
    F = w3.shape[1]
    R = ROWS
    n_blk = S // R
    n_tiles = D // LANES
    pairs = H // 2
    pairs_per_blk = pairs // n_blk
    assert E == LANES and n_blk == n_tiles and pairs % n_blk == 0 and H >= 8
    assert S % (GROUP_2 * R) == 0 and GROUP_2 % 2 == 0 and W1_SPLIT[-1] == D
    assert F % (LAST_PARTS * LANES) == 0 and n_tiles % LAST_PARTS == 0
    assert M % 8 == 0 and seg % 16 == 0 and S % (SEG_UNROLL * seg) == 0

    def copy(src, dst, i):
        return pltpu.make_async_copy(src, dst, sem_in.at[i])

    x_rows = [pl.ds(i * R, R) for i in range(3)]
    x_rows += [pl.ds(i * R, min(2 * R, S - i * R)) for i in range(3, n_blk, 2)]
    w1_rows = [slice(r0, r1) for r0, r1 in zip(W1_SPLIT, W1_SPLIT[1:])]
    cp_x = [copy(x_hbm.at[0, rs], xs.at[rs], i) for i, rs in enumerate(x_rows)]
    cp_w1 = [copy(w1_hbm.at[rs], w1.at[rs], n_blk + i) for i, rs in enumerate(w1_rows)]
    cp_w2, cp_w3, cp_w4, cp_gw, cp_mem = [
        copy(src, dst, n_blk + len(w1_rows) + i) for i, (src, dst) in enumerate(
            ((w2_hbm, w2), (w3_hbm, w3), (w4_hbm, w4), (gw_hbm, gw), (mem0_hbm, mem0)))]

    def slabs(i):
        return [(w, (m, i * pairs_per_blk + t))
                for m, w in enumerate((wq_hbm, wk_hbm, wv_hbm)) for t in range(pairs_per_blk)]

    def qkv_copies(i):
        return [pltpu.make_async_copy(w.bitcast(U32).at[:, p, :], wqkv.at[m * pairs + p],
                                      sem_qkv.at[m * pairs + p])
                for w, (m, p) in slabs(i)]

    def wo_copy(n):
        cols = pl.ds(pl.multiple_of(n * LANES, LANES), LANES)
        return pltpu.make_async_copy(wo_hbm.at[:, :, cols], wo.at[n], sem_wo.at[n])

    for cp in ([cp_x[0], cp_gw, cp_x[1]] + cp_w1 + cp_x[2:]
               + [cp_w2, cp_mem, cp_w3, cp_w4]):
        cp.start()

    def rows(i, offset=0):
        return pl.ds(pl.multiple_of(i * R + offset, 8), R)

    lhs = (lhs0, lhs1)
    hbuf[:, 0:HALO, :] = jnp.zeros((n_tiles, HALO, LANES), F32)
    hbuf[:, HALO + S:, :] = jnp.zeros((n_tiles, HALO, LANES), F32)

    def prepare1(i, slot, y=None):
        x = xs[rows(i), :].astype(F32)
        if y is not None:
            x = _during(y, x)
        logit = jnp.sum(x * gw[...].reshape(1, D).astype(F32), axis=-1, keepdims=True)
        gate[rows(i), :] = jnp.broadcast_to(jax.nn.sigmoid(logit), (R, LANES))
        lhs[slot][...] = _layernorm(x).astype(BF16)

    def store_h(i, pre):
        h = _gelu(pre)
        for n in range(n_tiles):
            hbuf[n, rows(i, HALO), :] = h[:, n * LANES:(n + 1) * LANES]

    cp_x[0].wait()
    cp_gw.wait()
    prepare1(0, 0)
    cp_x[1].wait()
    prepare1(1, 1)
    for c, (cp, ks) in enumerate(zip(cp_w1, w1_rows)):
        final = c == len(cp_w1) - 1
        cp.wait()
        for i in range(2):
            if final and i == 1:
                cp_x[2].wait()
            pre = _dot(lhs[i][:, ks], w1[ks, :])
            if c > 0:
                pre = bres[rows(i), :] + pre
            if final:
                store_h(i, pre)
            else:
                bres[rows(i), :] = pre
    prepare1(2, 0, pre)

    def step1(j, carry):
        for k in range(1, n_blk // 2):
            pl.when(j == k)(cp_x[k + 2].wait)
        for slot in range(2):
            i = 2 * j + slot
            pre = _dot(lhs[slot][...], w1[...])
            store_h(i, pre)
            prepare1(jnp.minimum(i + 1, n_blk - 1), 1 - slot, pre)
        return carry

    lax.fori_loop(1, n_blk // 2, step1, 0)

    def prepare2(i, slot, y=None):
        for n in range(n_tiles):
            shift = SHIFTS[n * len(SHIFTS) // n_tiles]
            part = hbuf[n, pl.ds(i * R + HALO + shift, R), :]
            if y is not None:
                part = _during(y, part)
            lhs[slot][:, n * LANES:(n + 1) * LANES] = part.astype(BF16)

    def step2(j, carry):
        x1 = None
        for t in range(GROUP_2):
            i = GROUP_2 * j + t
            hs = _dot(lhs[t % 2][...], w2[...])
            if x1 is not None:
                outbuf[rows(i - 1), :] = _layernorm(_during(hs, x1)).astype(BF16)
            x1 = xs[rows(i), :].astype(F32) + hs
            bres[rows(i), :] = x1
            prepare2(jnp.minimum(i + 1, n_blk - 1), 1 - t % 2, hs)
        outbuf[rows(i), :] = _layernorm(x1).astype(BF16)
        return carry

    cp_w2.wait()
    for cp in qkv_copies(0) + qkv_copies(1):
        cp.start()
    prepare2(0, 0)
    lax.fori_loop(0, n_blk // GROUP_2, step2, 0)

    def repack(j, k, dep):
        half = LANES // 2
        r = pl.multiple_of(k * LANES, LANES)
        w = _after(dep, wqkv[j, pl.ds(r, LANES), :])
        even = pltpu.bitcast(w << 16, F32).astype(BF16)
        odd = pltpu.bitcast(w & U32(0xFFFF0000), F32).astype(BF16)
        wqkv[j, pl.ds(r, half), :] = pltpu.bitcast(even, U32)
        wqkv[j, pl.ds(pl.multiple_of(r + half, half), half), :] = pltpu.bitcast(odd, U32)

    def mlp(i, q, parts):
        width = F // parts
        fs = pl.ds(pl.multiple_of(q * width, LANES), width)
        pre = _dot(outbuf[rows(i), :], w3[:, fs])
        todo = [(m * pairs + p, q * (n_tiles // parts) + t)
                for _, (m, p) in slabs(i) for t in range(n_tiles // parts)]
        for u, (j, k) in enumerate(todo):
            repack(j, k, _mark(pre, u * 2 * (width // LANES) // len(todo), 2))
        bres[rows(i), :] += _dot(_gelu(pre), w4[fs, :])

    def step3(i, carry):
        for cp in qkv_copies(i):
            cp.wait()
        mlp(i, 0, 1)
        wo_copy(i).start()

        @pl.when(i + 2 < n_blk)
        def _():
            for cp in qkv_copies(i + 2):
                cp.start()

        return carry

    cp_w3.wait()
    cp_w4.wait()
    lax.fori_loop(0, n_blk - 1, step3, 0)
    wo_copy(n_blk - 1).start()
    for cp in qkv_copies(n_blk - 1):
        cp.wait()
    lax.fori_loop(0, LAST_PARTS, lambda q, _: mlp(n_blk - 1, q, LAST_PARTS), None)
    for n in range(n_tiles):
        wo_copy(n).wait()

    def head_weight(m, h):
        j, off = m * pairs + h // 2, (h % 2) * (LANES // 2)
        w = jnp.concatenate(
            [wqkv[j, k * LANES + off:k * LANES + off + LANES // 2, :] for k in range(n_tiles)],
            axis=0)
        return pltpu.bitcast(w, BF16)

    row = lax.broadcasted_iota(jnp.int32, (L, L), 0)
    col = lax.broadcasted_iota(jnp.int32, (L, L), 1)
    mask = (row < M) | (row >= col)

    cp_mem.wait()
    hseg[0:M, :] = mem0[0].astype(F32)

    def step4(s, carry):
        tokens = pl.ds(pl.multiple_of(s * seg, seg), seg)
        hseg[M:L, :] = xs[tokens, :].astype(F32)
        qkv = {}
        probs = {}

        def project(h):
            hh = hseg[...]
            ws = [head_weight(m, h) for m in range(3)]
            if h == 0:
                k = D // 2
                oacc[:, 0:3 * E] = jnp.concatenate([_dot(hh[:, :k], w[:k]) for w in ws], axis=1)
                qkv[h] = [oacc[:, m * E:(m + 1) * E] + _dot(hh[:, k:], w[k:])
                          for m, w in enumerate(ws)]
            else:
                qkv[h] = [_dot(hh, w) for w in ws]

        def scores(h):
            q, k, _ = qkv[h]
            sc = jnp.where(mask, _dot_nt(q, k) * E ** (-0.5), -1000000000.0)
            e = jnp.exp(sc - jnp.max(sc, axis=-1, keepdims=True))
            probs[h] = e / jnp.sum(e, axis=-1, keepdims=True)

        def values(h):
            obuf[:, h * E:(h + 1) * E] = _dot(probs.pop(h), qkv.pop(h)[2])

        def out_part(h0, h1, n):
            return _dot(obuf[:, h0 * E:h1 * E], wo[n, h0:h1].reshape((h1 - h0) * E, LANES))

        for h in range(H):
            project(h)
            if h >= 1:
                scores(h - 1)
            if h >= 3:
                values(h - 3)
        late = {0: [(scores, H - 1), (values, H - 3)], 2: [(values, H - 2)], 3: [(values, H - 1)]}
        for n in range(n_tiles):
            oacc[:, n * LANES:(n + 1) * LANES] = out_part(0, H // 2, n)
            for fn, h in late.get(n, ()):
                fn(h)
        g = gate[tokens, :]
        for n in range(n_tiles):
            cols = slice(n * LANES, (n + 1) * LANES)
            o = oacc[:, cols] + out_part(H // 2, H, n)
            hseg[0:M, cols] = o[0:M]
            mixed = g * o[M:L] + (1.0 - g) * bres[tokens, cols]
            outbuf[tokens, cols] = mixed.astype(outbuf.dtype)
        pltpu.make_async_copy(outbuf.at[tokens], out_hbm.at[0, tokens], sem_out).start()
        return carry

    lax.fori_loop(0, S // seg, step4, 0, unroll=SEG_UNROLL)
    pltpu.make_async_copy(outbuf, out_hbm.at[0], sem_out).wait()


@functools.partial(jax.jit, static_argnames=("A_seg_len",))
def pallas_gated_mix__memory_aug_recurrent_mem_tr__mixer_s_mlp__prompt_kernel(
    A_x: jax.Array,
    A_mem0: jax.Array,
    A_Wq: jax.Array,
    A_Wk: jax.Array,
    A_Wv: jax.Array,
    A_Wo: jax.Array,
    A_seg_len: int,
    B_x: jax.Array,
    B_w1: jax.Array,
    B_w2: jax.Array,
    B_w3: jax.Array,
    B_w4: jax.Array,
    gate_w: jax.Array,
):
    del B_x
    batch, S, D = A_x.shape
    _, H, E = A_Wq.shape
    F = B_w3.shape[1]
    seg = int(A_seg_len)
    L = A_mem0.shape[1] + seg
    assert batch == 1 and A_x.dtype == BF16
    hbm = pl.BlockSpec(memory_space=pl.ANY)
    return pl.pallas_call(
        functools.partial(_kernel, seg=seg),
        out_shape=jax.ShapeDtypeStruct(A_x.shape, A_x.dtype),
        in_specs=[hbm] * 11,
        out_specs=hbm,
        scratch_shapes=[
            pltpu.VMEM((3 * H // 2, D, E), U32),
            pltpu.VMEM((D // LANES, H, E, LANES), BF16),
            pltpu.VMEM((D, D), BF16),
            pltpu.VMEM((D, D), BF16),
            pltpu.VMEM((D, F), BF16),
            pltpu.VMEM((F, D), BF16),
            pltpu.VMEM((S, D), BF16),
            pltpu.VMEM((D // LANES, S + 2 * HALO, LANES), F32),
            pltpu.VMEM((ROWS, D), BF16),
            pltpu.VMEM((ROWS, D), BF16),
            pltpu.VMEM((S, D), F32),
            pltpu.VMEM((S, LANES), F32),
            pltpu.VMEM((S, D), BF16),
            pltpu.VMEM((L, D), F32),
            pltpu.VMEM((L, H * E), F32),
            pltpu.VMEM((L, D), F32),
            pltpu.VMEM(A_mem0.shape, BF16),
            pltpu.VMEM(gate_w.shape, BF16),
            pltpu.SemaphoreType.DMA((S // ROWS + len(W1_SPLIT) + 4,)),
            pltpu.SemaphoreType.DMA((3 * H // 2,)),
            pltpu.SemaphoreType.DMA((D // LANES,)),
            pltpu.SemaphoreType.DMA(()),
        ],
        compiler_params=pltpu.CompilerParams(
            vmem_limit_bytes=120 * 1024 * 1024, disable_bounds_checks=True),
    )(A_x, A_mem0, A_Wq, A_Wk, A_Wv, A_Wo, B_w1, B_w2, B_w3, B_w4, gate_w)
```
